```python
import os as _os
_os.environ.setdefault("JAX_PLATFORMS", "cpu")
import jax
import jax.numpy as jnp

def _softmax(x, axis=-1):
    return jax.nn.softmax(x, axis=axis)
def _gelu(x):
    return jax.nn.gelu(x, approximate=True)
def _silu(x):
    return jax.nn.silu(x)
def _sigmoid(x):
    return jax.nn.sigmoid(x)
def _layernorm(x, axis=-1, eps=1e-5):
    m = jnp.mean(x, axis=axis, keepdims=True)
    v = jnp.var(x, axis=axis, keepdims=True)
    return (x - m) / jnp.sqrt(v + eps)
def _scatter_add(tgt, idx, src, axis=0):
    return tgt.at[idx].add(src)
def _segment_sum(src, seg, n):
    return jax.ops.segment_sum(src, seg, n)
class _Rng:
    def __init__(self, key):
        self._k = key
    def _next(self):
        self._k, sub = jax.random.split(self._k)
        return sub
    def normal(self, shape):
        return jax.random.normal(self._next(), shape, dtype=jnp.bfloat16)
    def randint(self, lo, hi, shape):
        return jax.random.randint(self._next(), shape, lo, hi, dtype=jnp.int32)
    def uniform(self, shape, lo=0.0, hi=1.0):
        return jax.random.uniform(self._next(), shape, jnp.bfloat16, lo, hi)
    def permutation(self, n):
        return jax.random.permutation(self._next(), n)


kernel_name = 'interleave_layers__ssm_conv_h3__linear_attn_block__prompt'

def setup_inputs():
    _rng = _Rng(jax.random.key(int.from_bytes(__import__("os").urandom(4), "little")))
    _w = (lambda a: (lambda t: t.astype(jnp.bfloat16) if jnp.issubdtype(t.dtype, jnp.floating) else t)(jnp.asarray(a)))
    def _A_setup():
        B, S, D = 1, 2048, 512
        ks = 4
        return {
            "q": _w((lambda *s: _rng.normal(s) * 0.05)(B, S, D)),
            "k": _w((lambda *s: _rng.normal(s) * 0.4)(B, S, D)),
            "v": _w((lambda *s: _rng.normal(s) * 0.4)(B, S, D)),
            "shift_k": _w((lambda *s: _rng.normal(s) * 0.4)(D, ks) * 0.5),
            "ssm_k": _w((lambda *s: _rng.normal(s) * 0.4)(D, S) * (1.0 / S ** 0.5)),
            "ssm_D": _w((lambda *s: _rng.normal(s) * 0.4)(D)),
        }
    _A_in = _A_setup()

    def _B_setup():
        B, S, D = 1, 2048, 512
        return {
            "x": _w((lambda *s: _rng.normal(s) * 0.05)(B, S, D)),
            "wqkv": _w((lambda *s: _rng.normal(s) * 0.1)(D, 3 * D)),
            "wo": _w((lambda *s: _rng.normal(s) * 0.1)(D, D)),
        }
    _B_in = _B_setup()

    return {
        "A_q": _A_in["q"],
        "A_k": _A_in["k"],
        "A_v": _A_in["v"],
        "A_shift_k": _A_in["shift_k"],
        "A_ssm_k": _A_in["ssm_k"],
        "A_ssm_D": _A_in["ssm_D"],
        "B_x": _B_in["x"],
        "B_wqkv": _B_in["wqkv"],
        "B_wo": _B_in["wo"],
    }

def reference(A_q, A_k, A_v, A_shift_k, A_ssm_k, A_ssm_D, B_x, B_wqkv, B_wo):
    def _A_ref(q, k, v, shift_k, ssm_k, ssm_D):
        B, S, D = q.shape
        ks = shift_k.shape[-1]
        k_pad = jnp.pad(k, ((0, 0), (ks - 1, 0), (0, 0)))
        k_shift = jnp.zeros_like(k)
        for t in range(ks):
            k_shift = k_shift + k_pad[:, t:t + S, :] * shift_k[:, ks - 1 - t][None, None, :]
        kv = k_shift * v
        L = 2 * S
        kv_pad = jnp.pad(kv, ((0, 0), (0, S), (0, 0)))
        kf_pad = jnp.pad(ssm_k, ((0, 0), (0, S)))
        kv_f = (lambda x, axes=(-2,-1): jnp.fft.rfft2(x.astype(jnp.float32), axes=axes))(kv_pad[:, None, :, :], axes=(1, 2))
        kf_f = (lambda x, axes=(-2,-1): jnp.fft.rfft2(x.astype(jnp.float32), axes=axes))(kf_pad[:, None, :], axes=(1, 2))
        kf_f = (lambda x, *d: x.transpose(*d))(kf_f, 1, 2, 0)
        y_f = kv_f * kf_f[None, :, :, :]
        y = (lambda x, s, axes=(-2,-1): jnp.fft.irfft2(x, s=s, axes=axes).astype(jnp.bfloat16))(y_f, (1, L), axes=(1, 2))[:, 0, :S, :]
        y = y + kv * ssm_D[None, None, :]
        return q * y

    def _B_ref(x, wqkv, wo):
        B, S, D = x.shape
        H = 32; Dh = D // H
        qkv = (lambda x, *d: x.transpose(*d))((x @ wqkv).reshape(B, S, 3, H, Dh), 2, 0, 3, 1, 4)
        q, k, v = qkv[0], qkv[1], qkv[2]
        phi = lambda t: jnp.where(t > 0, t + 1, jnp.exp(t)) + 1e-6
        pq, pk = phi(q), phi(k)
        kv = jnp.einsum("bhsd,bhse->bhde", pk, v)
        z = jnp.einsum("bhsd->bhd", pk)
        num = jnp.einsum("bhqd,bhde->bhqe", pq, kv)
        den = jnp.einsum("bhqd,bhd->bhq", pq, z)[..., None] + 1e-6
        o = num / den
        return (lambda x, *d: x.transpose(*d))(o, 0, 2, 1, 3).reshape(B, S, D) @ wo

    x = A_q
    x = x + _A_ref(_layernorm(x, axis=-1), A_k, A_v, A_shift_k, A_ssm_k, A_ssm_D)
    x = x + _B_ref(_layernorm(x, axis=-1), B_wqkv, B_wo)
    x = x + _A_ref(_layernorm(x, axis=-1), A_k, A_v, A_shift_k, A_ssm_k, A_ssm_D)
    x = x + _B_ref(_layernorm(x, axis=-1), B_wqkv, B_wo)
    return x
```

```python
import numpy as np
import jax
import jax.numpy as jnp
from jax import lax
import jax.experimental.pallas as pl
import jax.experimental.pallas.tpu as pltpu

S, D = 2048, 512
NU, UL = 8, 256
HL = 128
NG = 4
KPAD = 16
bf16, f32, u32 = jnp.bfloat16, jnp.float32, jnp.uint32
NT = (((1,), (1,)), ((), ()))
LAG = 0
PF = 0.5
PRSPLIT = 1
RL = 1
PLAG = 4
QC = 64
KC = 128


def _cos_pi512(idx):
    t = (256 - jnp.abs(idx)).astype(f32) * (np.pi / 512)
    t2 = t * t
    p = -2.5052108e-08
    for c in (2.7557319e-06, -1.9841270e-04, 8.3333333e-03, -1.6666667e-01, 1.0):
        p = p * t2 + c
    return p * t


def _dft_block(odd, part, transposed, scale):
    r = lax.broadcasted_iota(jnp.int32, (HL, HL), 1 if transposed else 0)
    m = lax.broadcasted_iota(jnp.int32, (HL, HL), 0 if transposed else 1)
    g2 = jnp.where(r < 64, 4 * r + 1, 4 * r - 253)
    idx = (g2 * (2 * m + odd) + (512 - 256 * part)) & 1023
    c = _cos_pi512(idx - 512)
    if scale != 1.0:
        c = c * scale
    return c


def _phi(t):
    return jnp.where(t > 0, t + 1.0, jnp.exp(t)) + 1e-6


def _ln(x):
    m = jnp.mean(x, axis=-1, keepdims=True)
    d = x - m
    v = jnp.mean(d * d, axis=-1, keepdims=True)
    return d * jnp.exp(-0.5 * jnp.log(v + 1e-5))


def _unp(w, i):
    return pltpu.unpack_elementwise(w, index=i, packed_dtype=bf16, unpacked_dtype=f32)


def _dot(a, b):
    return jnp.dot(a, b, preferred_element_type=f32)


def _w(x):
    return pltpu.bitcast(x, u32)


def _b(w):
    return pltpu.bitcast(w, bf16)


def _link(w, deps):
    if not deps:
        return w
    head = w[0:8]
    for d in deps:
        dw = d if d.dtype == u32 else pltpu.bitcast(d, u32)
        head = jnp.where(dw == jnp.uint32(0x7FC12345), dw, head)
    if w.shape[0] == 8:
        return head
    return jnp.concatenate([head, w[8:]], axis=0)


def _kernel(q_hbm, k_hbm, v_hbm, sk_hbm, h_hbm, dd_hbm, wqkv_hbm, wo_hbm, out_hbm,
            x0_s, k_s, v_s, sk_s, h_s, dd_s, w_s, wo_s, o_s,
            f_s, finv_s, c_s, wkt_s, u_s, hc_s, yf_s, prev_s, y_s, x_s, xn_s, qb_s, s_s,
            g_s, z_s, zbd_s, m_s,
            sem_u, sem_w):
    def lg(g):
        return pl.ds(g * 128, 128)

    def urows(n):
        return pl.ds(n * UL, UL)

    def cp_k(n, g):
        return pltpu.make_async_copy(k_hbm.at[urows(n), lg(g)],
                                     k_s.at[g, pl.ds(n * UL + KPAD, UL), :], sem_u.at[n])

    def cp_w(j, sem):
        if j < 12:
            return pltpu.make_async_copy(wqkv_hbm.at[:, lg(j)], w_s.at[j], sem)
        return pltpu.make_async_copy(wo_hbm.at[:, lg(j - 12)], wo_s.at[j - 12], sem)

    def out_cp(n, g):
        return pltpu.make_async_copy(o_s.at[g, urows(n), :], out_hbm.at[urows(n), lg(g)], sem_w.at[0])

    cp_sk = pltpu.make_async_copy(sk_hbm, sk_s, sem_w.at[2])
    cp_dd = pltpu.make_async_copy(dd_hbm, dd_s, sem_w.at[2])

    def copies(tag):
        kind, n = tag
        if kind == "kvh":
            return ([pltpu.make_async_copy(h_hbm.at[:, lg(2 * n + t)], h_s.at[2 * n + t], sem_u.at[n])
                     for t in range(2)]
                    + [cp_k(n, g) for g in range(NG)]
                    + [pltpu.make_async_copy(v_hbm.at[urows(n), lg(g)], v_s.at[g, urows(n), :], sem_u.at[n])
                       for g in range(NG)])
        if kind == "x":
            return [pltpu.make_async_copy(q_hbm.at[urows(n), lg(g)], x0_s.at[g, urows(n), :], sem_u.at[n])
                    for g in range(NG)]
        if kind == "w":
            if n == 2:
                return [cp_w(8 + j, sem_w.at[2]) for j in range(8)]
            return [cp_w(4 * n + j, sem_w.at[n]) for j in range(4)]
        raise ValueError(tag)

    def start(*tags):
        for t in tags:
            for c in copies(t):
                c.start()

    def wait(*tags):
        for t in tags:
            for c in copies(t):
                c.wait()

    kw = k_s.bitcast(u32)
    vw = v_s.bitcast(u32)
    xw = x0_s.bitcast(u32)
    hw = h_s.bitcast(u32)
    ww = w_s.bitcast(u32)
    wow = wo_s.bitcast(u32)
    ow = o_s.bitcast(u32)
    fw = f_s.bitcast(u32)
    fiw = finv_s.bitcast(u32)
    wktw = wkt_s.bitcast(u32)
    yfw = yf_s.bitcast(u32)
    xnw = xn_s.bitcast(u32)
    qbw = qb_s.bitcast(u32)
    sw_ = s_s.bitcast(u32)
    zbw = zbd_s.bitcast(u32)
    mw = m_s.bitcast(u32)

    def spread(parts, deps):
        k = len(parts)
        parts = [_link(p, list(deps[i::k])) for i, p in enumerate(parts)]
        return jnp.concatenate([_b(p) for p in parts], axis=1)

    def wcat(ref, j0, deps=()):
        return spread([ref[j0 + j] for j in range(NG)], deps)

    def lhs_cat(parts, deps):
        parts = [_link(parts[0], deps)] + list(parts[1:])
        return jnp.concatenate([_b(p) for p in parts], axis=1) if len(parts) > 1 else _b(parts[0])

    state = {"toks": [], "post": {}}

    def node(fn, fill=()):
        i = len(state["toks"])
        deps = []
        if LAG and i - LAG >= 0 and state["toks"][i - LAG] is not None:
            deps.append(state["toks"][i - LAG])
        deps += state["post"].pop(i, [])
        for f in fill:
            t = f()
            if t is not None:
                deps.append(t)
        tok, post = fn(deps)
        state["toks"].append(tok)
        if post:
            state["post"].setdefault(i + PLAG, []).extend(post)

    def barrier():
        state["toks"] = []
        state["post"] = {}

    def fwd4(xe, xo, deps):
        fe0 = _b(_link(fw[0, 0], deps))
        er = _dot(fe0, xe)
        pr_ = _dot(_b(fw[1, 0]), xo)
        ei = _dot(_b(fw[0, 1]), xe)
        pi_ = _dot(_b(fw[1, 1]), xo)
        return er, pr_, ei, pi_

    def st_pos(ref, g, n, c, val):
        for r in range(8):
            ref[r, g, n, c] = val[r * 16:(r + 1) * 16]

    def fu(n, gs):
        def fn(deps):
            post = []
            w0 = n * HL
            tok = None
            for g in gs:
                wg = c_s[:, lg(g)]
                W0 = kw[g, pl.ds(w0 + 8, HL), :]
                W1 = kw[g, pl.ds(w0 + 7, HL), :]
                W2 = kw[g, pl.ds(w0 + 6, HL), :]
                e0, o0, e1, o1, o2 = _unp(W0, 0), _unp(W0, 1), _unp(W1, 0), _unp(W1, 1), _unp(W2, 1)
                V = vw[g, pl.ds(w0, HL), :]
                ue = (wg[0:1] * e0 + wg[1:2] * o1 + wg[2:3] * e1 + wg[3:4] * o2) * _unp(V, 0)
                uo = (wg[0:1] * o0 + wg[1:2] * e0 + wg[2:3] * o1 + wg[3:4] * e1) * _unp(V, 1)
                er, pr_, ei, pi_ = fwd4(ue.astype(bf16), uo.astype(bf16), deps)
                deps = []
                st_pos(u_s, g, n, 0, er + pr_)
                st_pos(u_s, g, n, 2, er - pr_)
                st_pos(u_s, g, n, 1, ei + pi_)
                last = ei - pi_
                st_pos(u_s, g, n, 3, last)
                tok = last[HL - 8:]
                post.append(tok)
            return tok, post[:-1]
        return fn

    def fh(n, gs):
        def fn(deps):
            post = []
            tok = None
            for g in gs:
                es, os_ = [], []
                for t in range(2):
                    ht = _b(hw[2 * n + t, pl.ds(g * 64, 64), :]).T
                    W = _w(ht)
                    es.append(_unp(W, 0))
                    os_.append(_unp(W, 1))
                he = jnp.concatenate(es, axis=0).astype(bf16)
                ho = jnp.concatenate(os_, axis=0).astype(bf16)
                er, pr_, ei, pi_ = fwd4(he, ho, deps)
                deps = []
                if n == 0:
                    er = er + c_s[pl.ds(4, 1), lg(g)]
                for x, (c, d) in enumerate(((er + pr_, ei + pi_), (er - pr_, ei - pi_))):
                    st_pos(hc_s, g, n, 3 * x + 0, c)
                    st_pos(hc_s, g, n, 3 * x + 1, d - c)
                    last = c + d
                    st_pos(hc_s, g, n, 3 * x + 2, last)
                tok = last[HL - 8:]
                post.append(tok)
            return tok, post[:-1]
        return fn

    def pr_step(q, p):
        rg2, g = p % 8, p // 8
        sign = 1 if rg2 < 4 else -1
        m0, m1 = 2 * q, 2 * q + 1
        ys = []

        def tok_of(*vals):
            tk = None
            for v in vals:
                b = pltpu.bitcast(v, u32)
                tk = b if tk is None else tk | b
            return tk[0:8] | tk[8:16]

        def xpart(x):
            acc = {}
            hprev = None
            for a in range(m1 + 1):
                ua = u_s[rg2, g, a, 2 * x]
                ub = u_s[rg2, g, a, 2 * x + 1]
                uu = (ua + ub, ua, ub)
                if hprev is None:
                    hprev = [hc_s[rg2, g, m1 - a, 3 * x + t] for t in range(3)]
                h1 = hprev
                h0 = [hc_s[rg2, g, m0 - a, 3 * x + t] for t in range(3)] if a <= m0 else None
                for t in range(3):
                    p1 = uu[t] * h1[t]
                    acc[(1, t)] = p1 if a == 0 else acc[(1, t)] + p1
                    if h0 is not None:
                        p0 = uu[t] * h0[t]
                        acc[(0, t)] = p0 if a == 0 else acc[(0, t)] + p0
                hprev = h0
            ys.append([(acc[(i, 0)] - acc[(i, 2)], acc[(i, 0)] + acc[(i, 1)]) for i in range(2)])

        def fa():
            xpart(0)
            return tok_of(ys[0][0][0], ys[0][0][1], ys[0][1][0], ys[0][1][1])

        def fb():
            if not ys:
                xpart(0)
            xpart(1)
            ab = []
            for i in range(2):
                (r1, i1), (r2, i2) = ys[0][i], ys[1][i]
                ab.append((r1 + r2, i1 + i2, r1 - r2, i1 - i2))

            def win(cur, prv):
                if prv is None:
                    return cur
                o = []
                for t in range(2):
                    cr, ci, pr_, pi_ = cur[2 * t], cur[2 * t + 1], prv[2 * t], prv[2 * t + 1]
                    o += [cr + pi_, ci - pr_] if sign > 0 else [cr - pi_, ci + pr_]
                return o
            prv0 = None if q == 0 else [prev_s[q - 1, rg2, g, t] for t in range(4)]
            w = (win(ab[0], prv0), win(ab[1], ab[0]))
            if q < 3:
                for t in range(4):
                    prev_s[q, rg2, g, t] = ab[1][t]
            for i in range(2):
                m = 2 * q + i
                for t in range(2):
                    yf_s[m, t, g, pl.ds(rg2 * 16, 16), :] = w[i][2 * t].astype(bf16)
                    yf_s[m, t, g, pl.ds(HL + rg2 * 16, 16), :] = w[i][2 * t + 1].astype(bf16)
            return tok_of(w[1][0], w[1][1])
        return [fa, fb] if (PRSPLIT and q > 0) else [fb]

    class PRQ:
        def __init__(self, q):
            self.q, self.p = q, 0

        def take(self, k):
            out = [f for p in range(self.p, min(32, self.p + k)) for f in pr_step(self.q, p)]
            self.p = min(32, self.p + k)
            return out

    def lnln(n, layer, half, x):
        rows = pl.ds(n * UL + half * HL, HL)
        x1 = x + _ln(x) * y_s[rows, :]
        x_s[rows, :] = x1
        xn = _ln(x1)
        for g in range(NG):
            xn_s[layer, n, g, pl.ds(half * HL, HL), :] = xn[:, g * 128:(g + 1) * 128].astype(bf16)
        return xn[HL - 8:, 384:512]

    def inv(n, t):
        def fn(deps):
            fi = lhs_cat([fiw[t, 0], fiw[t, 1]], deps)
            ys = [_dot(fi, _b(yfw[n, t, g])) for g in range(NG)]
            y = jnp.concatenate(ys, axis=1)
            y_s[pl.ds(n * UL + t * HL, HL), :] = y
            x = jnp.concatenate([_unp(xw[g, pl.ds(n * HL, HL), :], t) for g in range(NG)], axis=1)
            ptok = lnln(n, 0, t, x)
            return ys[3][HL - 8:], [ptok]
        return fn

    def xn_full(layer, n, deps=()):
        return spread([xnw[layer, n, g] for g in range(NG)], deps)

    def qp(n, layer, c):
        def fn(deps):
            rr = pl.ds(c * QC // 2, QC // 2)
            x = lhs_cat([xnw[layer, n, g, rr, :] for g in range(NG)], [] if RL else deps)
            q = _dot(x, wcat(ww, 0, deps if RL else ()))
            for g in range(NG):
                qb_s[layer, n, g, pl.ds(c * QC, QC), :] = q[:, g * 128:(g + 1) * 128].astype(bf16)
            return q[QC - 8:, 384:512], []
        return fn

    pk_stash = {}

    def ktp(n, layer, c):
        def fn(deps):
            rr = pl.ds(c * KC // 2, KC // 2)
            wk = lhs_cat([wktw[g, rr, :] for g in range(NG)], deps[0::2] if RL else deps)
            if RL and len(deps) > 1:
                p0 = xnw[layer, n, 0]
                p0 = jnp.concatenate([p0[:64], _link(p0[64:], deps[1::2])], axis=0)
                xr = jnp.concatenate([_b(p0)] + [_b(xnw[layer, n, g]) for g in range(1, NG)], axis=1)
            else:
                xr = xn_full(layer, n)
            kt = lax.dot_general(wk, xr, NT, preferred_element_type=f32)
            pk = _phi(kt)
            zz = pk[:, 0:128] + pk[:, 128:256]
            rs = pl.ds(c * KC, KC)
            if n == 0:
                z_s[rs, :] = zz
            else:
                z_s[rs, :] += zz
            pk_stash[(n, layer, c)] = pk.astype(bf16)
            return kt[KC - 8:, 128:256], []
        return fn

    def gp(n, layer, c):
        def fn(deps):
            pk = pk_stash.pop((n, layer, c))
            gg = _dot(pk, xn_full(layer, n, deps))
            rs = pl.ds(c * KC, KC)
            if n == 0:
                g_s[rs, :] = gg
                return gg[KC - 8:, 384:512], []
            new = g_s[rs, :] + gg
            g_s[rs, :] = new
            return gg[KC - 8:, 384:512], [new[KC - 8:, 384:512]]
        return fn

    def qkg_nodes(n, layer):
        nq, nk = UL // QC, D // KC
        qs = [qp(n, layer, c) for c in range(nq)]
        ks = [ktp(n, layer, c) for c in range(nk)]
        gs = [gp(n, layer, c) for c in range(nk)]
        out = []
        for c in range(nk):
            out.append(ks[c])
            if c > 0:
                out.append(gs[c - 1])
            lo, hi = c * nq // nk, (c + 1) * nq // nk
            out += qs[lo:hi]
        out.append(gs[nk - 1])
        return out

    def kg_nodes(n, layer):
        nk = D // KC
        out = []
        for c in range(nk):
            out.append(ktp(n, layer, c))
            if c > 0:
                out.append(gp(n, layer, c - 1))
        out.append(gp(n, layer, nk - 1))
        return out

    def q_nodes(n, layer):
        return [qp(n, layer, c) for c in range(UL // QC)]

    def finalize():
        ri = lax.broadcasted_iota(jnp.int32, (128, 128), 0) >> 4
        ci = lax.broadcasted_iota(jnp.int32, (128, 128), 1) >> 4
        mask = ri == ci
        z = jnp.sum(z_s[...], axis=1, keepdims=True)
        for g in range(NG):
            rs = pl.ds(g * 128, 128)
            zbd_s[g] = jnp.where(mask, z[g * 128:(g + 1) * 128], 0.0).astype(bf16)
            kv = _dot(g_s[rs, :].astype(bf16), _b(ww[8 + g]))
            kv = jnp.where(mask, kv, 0.0).astype(bf16)
            for j in range(NG):
                m_s[j, rs, :] = _dot(kv, _b(wow[j, pl.ds(g * 64, 64), :])).astype(bf16)

    def denp(n, layer, half):
        def fn(deps):
            rr = pl.ds(half * 64, 64)
            tok = None
            for g in range(NG):
                pq = _phi(_b(qbw[layer, n, g, rr, :]).astype(f32))
                den = _dot(pq.astype(bf16), _b(_link(zbw[g], deps))) + 1e-6
                deps = []
                s_s[n, g, pl.ds(half * HL, HL), :] = (pq * pl.reciprocal(den, approx=True)).astype(bf16)
                tok = den[HL - 8:]
            return tok, []
        return fn

    att_stash = {}

    def outp(n, layer, c):
        def fn(deps):
            rr = pl.ds(c * QC // 2, QC // 2)
            s = lhs_cat([sw_[n, g, rr, :] for g in range(NG)], [] if RL else deps)
            a = _dot(s, wcat(mw, 0, deps if RL else ()))
            x2 = x_s[pl.ds(n * UL + c * QC, QC), :] + a
            att_stash.setdefault(n, []).append(x2)
            post = []
            per = HL // QC
            if (c + 1) % per == 0:
                half = c // per
                xh = jnp.concatenate(att_stash[n][half * per:(half + 1) * per], axis=0)
                if layer == 0:
                    post.append(lnln(n, 1, half, xh))
                elif half == 1:
                    xe = jnp.concatenate(att_stash[n][:per], axis=0)
                    pkd = pltpu.pack_elementwise([xe, xh], packed_dtype=bf16)
                    for g in range(NG):
                        ow[g, pl.ds(n * HL, HL), :] = pkd[:, g * 128:(g + 1) * 128]
                    post.append(pkd[HL - 8:, 384:512])
                if half == 1:
                    del att_stash[n]
            return a[QC - 8:, 384:512], post
        return fn

    def p2_nodes(n, layer):
        no = UL // QC
        return [denp(n, layer, 0), denp(n, layer, 1)] + [outp(n, layer, c) for c in range(no)]

    def gen_finv():
        for odd in range(2):
            for part in range(2):
                finv_s[odd, part] = _dft_block(odd, part, True, 1.0 / UL).astype(bf16)

    def make_wkt():
        wkt = wcat(ww, 4).T
        for g in range(NG):
            wkt_s[g] = wkt[:, g * 128:(g + 1) * 128]

    def merge(*lists):
        items = []
        for li, l in enumerate(lists):
            lo, hi = 0.0, 1.0
            if isinstance(l, tuple):
                l, lo, hi = l
            for j, x in enumerate(l):
                items.append((lo + (hi - lo) * (j + 0.5) / len(l), li, x))
        items.sort(key=lambda t: (t[0], t[1]))
        return [x for _, _, x in items]

    def run(nodes, fillers=(), lo=0.0, hi=1.0):
        fillers = list(fillers)
        nn = len(nodes)
        i0, i1 = int(lo * nn), max(int(lo * nn) + 1, int(round(hi * nn)))
        for i, fn in enumerate(nodes):
            if i < i0 or i >= i1 or not fillers:
                node(fn)
                continue
            k = -(-len(fillers) // (i1 - i))
            node(fn, fillers[:k])
            fillers = fillers[k:]
        assert not fillers

    def fufh_nodes(n):
        return [fh(n, (0, 1)), fu(n, (0, 1)), fh(n, (2, 3)), fu(n, (2, 3))]

    def inv_nodes(n):
        return [inv(n, 0), inv(n, 1)]

    cp_sk.start()
    cp_dd.start()
    start(("kvh", 0), ("kvh", 1))
    for odd in range(2):
        for part in range(2):
            f_s[odd, part] = _dft_block(odd, part, False, 1.0).astype(bf16)
    for g in range(NG):
        k_s[g, pl.ds(0, KPAD), :] = jnp.zeros((KPAD, 128), bf16)
    cp_sk.wait()
    cp_dd.wait()
    c_s[pl.ds(0, 4), :] = sk_s[...].astype(f32)
    c_s[pl.ds(4, 1), :] = dd_s[...].astype(f32).reshape(1, D)
    c_s[pl.ds(5, 3), :] = jnp.zeros((3, D), f32)

    prq = [PRQ(q) for q in range(4)]
    wait(("kvh", 0))
    start(("kvh", 2), ("x", 0), ("w", 1))
    run(fufh_nodes(0))
    wait(("kvh", 1))
    start(("w", 0), ("x", 1), ("kvh", 3))
    gen_finv()
    run(fufh_nodes(1))
    wait(("kvh", 2))
    start(("x", 2), ("kvh", 4))
    run(fufh_nodes(2), prq[0].take(32))
    wait(("x", 0), ("w", 1))
    make_wkt()
    run(inv_nodes(0))
    wait(("x", 1), ("w", 0), ("kvh", 3))
    start(("x", 3), ("kvh", 5), ("kvh", 6))
    run(merge((inv_nodes(1), 0.0, 0.3), (fufh_nodes(3), 0.0, 0.6), kg_nodes(0, 0)))
    wait(("x", 2), ("kvh", 4))
    start(("x", 4), ("kvh", 7))
    run(merge(kg_nodes(1, 0), q_nodes(0, 0), fufh_nodes(4)) + inv_nodes(2), prq[1].take(32), 0.0, 0.88)
    wait(("x", 3), ("kvh", 5))
    start(("x", 5), ("w", 2))
    run(merge((inv_nodes(3), 0.0, 0.3), (fufh_nodes(5), 0.0, 0.4), kg_nodes(2, 0), q_nodes(1, 0)),
        prq[2].take(10), 0.5, 1.0)
    wait(("kvh", 6), ("x", 4))
    start(("x", 6))
    run(merge(kg_nodes(3, 0), q_nodes(2, 0), fufh_nodes(6)) + inv_nodes(4), prq[2].take(22), 0.0, 0.88)
    wait(("kvh", 7), ("x", 5))
    start(("x", 7))
    run(merge((inv_nodes(5), 0.0, 0.3), (fufh_nodes(7), 0.0, 0.4), kg_nodes(4, 0), q_nodes(3, 0)),
        prq[3].take(9), 0.5, 1.0)
    wait(("x", 6))
    run(merge(kg_nodes(5, 0), q_nodes(4, 0), q_nodes(5, 0)) + inv_nodes(6), prq[3].take(23), 0.0, 0.88)
    wait(("x", 7))
    run(merge((inv_nodes(7), 0.0, 0.3), kg_nodes(6, 0), q_nodes(6, 0)))
    wait(("w", 2))
    run(merge(kg_nodes(7, 0), q_nodes(7, 0)))
    barrier()
    finalize()

    run(p2_nodes(0, 0))
    for n in range(NU):
        if n + 1 < NU:
            run(merge((p2_nodes(n + 1, 0), 0.0, PF), qkg_nodes(n, 1)))
        else:
            run(qkg_nodes(n, 1))
    barrier()
    finalize()

    run(p2_nodes(0, 1)[:2])
    for n in range(NU):
        nxt = p2_nodes(n + 1, 1)[:2] if n + 1 < NU else []
        run(merge(p2_nodes(n, 1)[2:], nxt) if nxt else p2_nodes(n, 1)[2:])
        for g in range(NG):
            out_cp(n, g).start()
    for n in range(NU):
        for g in range(NG):
            out_cp(n, g).wait()


@jax.jit
def pallas_interleave_layers__ssm_conv_h3__linear_attn_block__prompt_kernel(
        A_q, A_k, A_v, A_shift_k, A_ssm_k, A_ssm_D, B_x, B_wqkv, B_wo):
    del B_x
    any_spec = pl.BlockSpec(memory_space=pl.ANY)
    scratch = [
        pltpu.VMEM((NG, S, 128), bf16),
        pltpu.VMEM((NG, S + KPAD, 128), bf16),
        pltpu.VMEM((NG, S, 128), bf16),
        pltpu.VMEM((4, D), bf16),
        pltpu.VMEM((2 * NU, D, 128), bf16),
        pltpu.VMEM((D,), bf16),
        pltpu.VMEM((12, D, 128), bf16),
        pltpu.VMEM((NG, D, 128), bf16),
        pltpu.VMEM((NG, S, 128), bf16),
        pltpu.VMEM((2, 2, HL, HL), bf16),
        pltpu.VMEM((2, 2, HL, HL), bf16),
        pltpu.VMEM((8, D), f32),
        pltpu.VMEM((NG, D, 128), bf16),
        pltpu.VMEM((8, NG, NU, 4, 16, 128), f32),
        pltpu.VMEM((8, NG, NU, 6, 16, 128), f32),
        pltpu.VMEM((NU, 2, NG, UL, 128), bf16),
        pltpu.VMEM((3, 8, NG, 4, 16, 128), f32),
        pltpu.VMEM((S, D), f32),
        pltpu.VMEM((S, D), f32),
        pltpu.VMEM((2, NU, NG, UL, 128), bf16),
        pltpu.VMEM((2, NU, NG, UL, 128), bf16),
        pltpu.VMEM((NU, NG, UL, 128), bf16),
        pltpu.VMEM((D, D), f32),
        pltpu.VMEM((D, 128), f32),
        pltpu.VMEM((NG, 128, 128), bf16),
        pltpu.VMEM((NG, D, 128), bf16),
        pltpu.SemaphoreType.DMA((NU,)),
        pltpu.SemaphoreType.DMA((3,)),
    ]
    out = pl.pallas_call(
        _kernel,
        out_shape=jax.ShapeDtypeStruct((S, D), bf16),
        in_specs=[any_spec] * 8,
        out_specs=any_spec,
        scratch_shapes=scratch,
        compiler_params=pltpu.CompilerParams(vmem_limit_bytes=110 * 1024 * 1024),
    )(A_q.reshape(S, D), A_k.reshape(S, D), A_v.reshape(S, D), A_shift_k.T, A_ssm_k,
      A_ssm_D, B_wqkv, B_wo)
    return out.reshape(1, S, D)
```

```python
import numpy as np
import jax
import jax.numpy as jnp
from jax import lax
import jax.experimental.pallas as pl
import jax.experimental.pallas.tpu as pltpu

S, D = 2048, 512
NU, UL = 8, 256
HL = 128
NG = 4
KPAD = 16
bf16, f32, u32 = jnp.bfloat16, jnp.float32, jnp.uint32
NT = (((1,), (1,)), ((), ()))
LAG = 0
PF = 0.5
PRSPLIT = 1
RL = 1
FWD = 3
PR2A = 14
PR1A = 14
PLAG = 4
QC = 64
KC = 128


def _cos_pi512(idx):
    t = (256 - jnp.abs(idx)).astype(f32) * (np.pi / 512)
    t2 = t * t
    p = -2.5052108e-08
    for c in (2.7557319e-06, -1.9841270e-04, 8.3333333e-03, -1.6666667e-01, 1.0):
        p = p * t2 + c
    return p * t


def _dft_block(odd, part, transposed, scale):
    r = lax.broadcasted_iota(jnp.int32, (HL, HL), 1 if transposed else 0)
    m = lax.broadcasted_iota(jnp.int32, (HL, HL), 0 if transposed else 1)
    g2 = jnp.where(r < 64, 4 * r + 1, 4 * r - 253)
    idx = (g2 * (2 * m + odd) + (512 - 256 * part)) & 1023
    c = _cos_pi512(idx - 512)
    if scale != 1.0:
        c = c * scale
    return c


def _phi(t):
    return jnp.where(t > 0, t + 1.0, jnp.exp(t)) + 1e-6


def _ln(x):
    m = jnp.mean(x, axis=-1, keepdims=True)
    d = x - m
    v = jnp.mean(d * d, axis=-1, keepdims=True)
    return d * jnp.exp(-0.5 * jnp.log(v + 1e-5))


def _unp(w, i):
    return pltpu.unpack_elementwise(w, index=i, packed_dtype=bf16, unpacked_dtype=f32)


def _dot(a, b):
    return jnp.dot(a, b, preferred_element_type=f32)


def _w(x):
    return pltpu.bitcast(x, u32)


def _b(w):
    return pltpu.bitcast(w, bf16)


def _link(w, deps):
    if not deps:
        return w
    head = w[0:8]
    for d in deps:
        dw = d if d.dtype == u32 else pltpu.bitcast(d, u32)
        head = jnp.where(dw == jnp.uint32(0x7FC12345), dw, head)
    if w.shape[0] == 8:
        return head
    return jnp.concatenate([head, w[8:]], axis=0)


def _kernel(q_hbm, k_hbm, v_hbm, sk_hbm, h_hbm, dd_hbm, wqkv_hbm, wo_hbm, out_hbm,
            x0_s, k_s, v_s, sk_s, h_s, dd_s, w_s, wo_s, o_s,
            f_s, finv_s, c_s, wkt_s, u_s, hc_s, yf_s, prev_s, y_s, x_s, xn_s, qb_s, s_s,
            g_s, z_s, zbd_s, m_s,
            sem_u, sem_w):
    def lg(g):
        return pl.ds(g * 128, 128)

    def urows(n):
        return pl.ds(n * UL, UL)

    def cp_w(j, sem):
        if j < 12:
            return pltpu.make_async_copy(wqkv_hbm.at[:, lg(j)], w_s.at[j], sem)
        return pltpu.make_async_copy(wo_hbm.at[:, lg(j - 12)], wo_s.at[j - 12], sem)

    def out_cp(n, g):
        return pltpu.make_async_copy(o_s.at[g, urows(n), :], out_hbm.at[urows(n), lg(g)], sem_w.at[0])

    cp_sk = pltpu.make_async_copy(sk_hbm, sk_s, sem_w.at[2])
    cp_dd = pltpu.make_async_copy(dd_hbm, dd_s, sem_w.at[2])

    def copies(tag):
        kind, n = tag
        if kind in ("kvh", "kv01", "kv23", "h"):
            sem = {"kvh": sem_u.at[n], "kv01": sem_u.at[n], "kv23": sem_w.at[5], "h": sem_w.at[6]}[kind]
            gs = {"kvh": (0, 1, 2, 3), "kv01": (0, 1), "kv23": (2, 3), "h": ()}[kind]
            out = []
            for g in gs:
                out.append(pltpu.make_async_copy(k_hbm.at[urows(n), lg(g)],
                                                 k_s.at[g, pl.ds(n * UL + KPAD, UL), :], sem))
                out.append(pltpu.make_async_copy(v_hbm.at[urows(n), lg(g)], v_s.at[g, urows(n), :], sem))
            if kind in ("kvh", "h"):
                out += [pltpu.make_async_copy(h_hbm.at[:, lg(2 * n + t)], h_s.at[2 * n + t], sem)
                        for t in range(2)]
            return out
        if kind in ("xa", "xb", "xc"):
            sem = {"xa": sem_w.at[3], "xb": sem_w.at[4], "xc": sem_w.at[5]}[kind]
            return [pltpu.make_async_copy(q_hbm.at[urows(n), lg(g)], x0_s.at[g, urows(n), :], sem)
                    for g in range(NG)]
        if kind == "w":
            if n == 2:
                return [cp_w(8 + j, sem_w.at[2]) for j in range(8)]
            return [cp_w(4 * n + j, sem_w.at[n]) for j in range(4)]
        raise ValueError(tag)

    def start(*tags):
        for t in tags:
            for c in copies(t):
                c.start()

    def wait(*tags):
        for t in tags:
            for c in copies(t):
                c.wait()

    kw = k_s.bitcast(u32)
    vw = v_s.bitcast(u32)
    xw = x0_s.bitcast(u32)
    hw = h_s.bitcast(u32)
    ww = w_s.bitcast(u32)
    wow = wo_s.bitcast(u32)
    ow = o_s.bitcast(u32)
    fw = f_s.bitcast(u32)
    fiw = finv_s.bitcast(u32)
    wktw = wkt_s.bitcast(u32)
    yfw = yf_s.bitcast(u32)
    xnw = xn_s.bitcast(u32)
    qbw = qb_s.bitcast(u32)
    sw_ = s_s.bitcast(u32)
    zbw = zbd_s.bitcast(u32)
    mw = m_s.bitcast(u32)

    def spread(parts, deps):
        k = len(parts)
        parts = [_link(p, list(deps[i::k])) for i, p in enumerate(parts)]
        return jnp.concatenate([_b(p) for p in parts], axis=1)

    def wcat(ref, j0, deps=()):
        return spread([ref[j0 + j] for j in range(NG)], deps)

    def lhs_cat(parts, deps):
        parts = [_link(parts[0], deps)] + list(parts[1:])
        return jnp.concatenate([_b(p) for p in parts], axis=1) if len(parts) > 1 else _b(parts[0])

    state = {"toks": [], "post": {}}

    def node(fn, fill=()):
        i = len(state["toks"])
        deps = []
        if LAG and i - LAG >= 0 and state["toks"][i - LAG] is not None:
            deps.append(state["toks"][i - LAG])
        deps += state["post"].pop(i, [])
        pre = state["toks"][i - FWD] if (FWD and i - FWD >= 0) else None
        for f in fill:
            t = f(pre)
            if t is not None:
                deps.append(t)
        tok, post = fn(deps)
        state["toks"].append(tok)
        if post:
            state["post"].setdefault(i + PLAG, []).extend(post)

    def barrier():
        state["toks"] = []
        state["post"] = {}

    def fwd4(xe, xo, deps):
        fe0 = _b(_link(fw[0, 0], deps))
        er = _dot(fe0, xe)
        pr_ = _dot(_b(fw[1, 0]), xo)
        ei = _dot(_b(fw[0, 1]), xe)
        pi_ = _dot(_b(fw[1, 1]), xo)
        return er, pr_, ei, pi_

    def st_pos(ref, g, n, c, val):
        for r in range(8):
            ref[r, g, n, c] = val[r * 16:(r + 1) * 16]

    def fu(n, gs):
        def fn(deps):
            post = []
            w0 = n * HL
            tok = None
            for g in gs:
                wg = c_s[:, lg(g)]
                W0 = kw[g, pl.ds(w0 + 8, HL), :]
                W1 = kw[g, pl.ds(w0 + 7, HL), :]
                W2 = kw[g, pl.ds(w0 + 6, HL), :]
                e0, o0, e1, o1, o2 = _unp(W0, 0), _unp(W0, 1), _unp(W1, 0), _unp(W1, 1), _unp(W2, 1)
                V = vw[g, pl.ds(w0, HL), :]
                ue = (wg[0:1] * e0 + wg[1:2] * o1 + wg[2:3] * e1 + wg[3:4] * o2) * _unp(V, 0)
                uo = (wg[0:1] * o0 + wg[1:2] * e0 + wg[2:3] * o1 + wg[3:4] * e1) * _unp(V, 1)
                er, pr_, ei, pi_ = fwd4(ue.astype(bf16), uo.astype(bf16), deps)
                deps = []
                st_pos(u_s, g, n, 0, er + pr_)
                st_pos(u_s, g, n, 2, er - pr_)
                st_pos(u_s, g, n, 1, ei + pi_)
                last = ei - pi_
                st_pos(u_s, g, n, 3, last)
                tok = last[HL - 8:]
                post.append(tok)
            return tok, post[:-1]
        return fn

    def fh(n, gs):
        def fn(deps):
            post = []
            tok = None
            for g in gs:
                es, os_ = [], []
                for t in range(2):
                    ht = _b(hw[2 * n + t, pl.ds(g * 64, 64), :]).T
                    W = _w(ht)
                    es.append(_unp(W, 0))
                    os_.append(_unp(W, 1))
                he = jnp.concatenate(es, axis=0).astype(bf16)
                ho = jnp.concatenate(os_, axis=0).astype(bf16)
                er, pr_, ei, pi_ = fwd4(he, ho, deps)
                deps = []
                if n == 0:
                    er = er + c_s[pl.ds(4, 1), lg(g)]
                for x, (c, d) in enumerate(((er + pr_, ei + pi_), (er - pr_, ei - pi_))):
                    st_pos(hc_s, g, n, 3 * x + 0, c)
                    st_pos(hc_s, g, n, 3 * x + 1, d - c)
                    last = c + d
                    st_pos(hc_s, g, n, 3 * x + 2, last)
                tok = last[HL - 8:]
                post.append(tok)
            return tok, post[:-1]
        return fn

    def pr_step(outs_m, p):
        rg2, g = p % 8, p // 8
        sign = 1 if rg2 < 4 else -1
        no = len(outs_m)
        ys = {}
        outs = {}

        def xpart(h, x, pre):
            hs = pl.ds(8 * h, 8)
            acc = {}
            hcache = {}

            def hget(j):
                if j not in hcache:
                    hcache[j] = [hc_s[rg2, g, j, 3 * x + t, hs, :] for t in range(3)]
                return hcache[j]
            for a in range(outs_m[-1] + 1):
                ua = u_s[rg2, g, a, 2 * x, hs, :]
                ub = u_s[rg2, g, a, 2 * x + 1, hs, :]
                if a == 0 and pre is not None:
                    ua = jnp.where(pltpu.bitcast(pre, u32) == jnp.uint32(0x7FC12345), pre, ua)
                uu = (ua + ub, ua, ub)
                for i in reversed(range(no)):
                    m = outs_m[i]
                    if a > m:
                        continue
                    hh = hget(m - a)
                    for t in range(3):
                        pp = uu[t] * hh[t]
                        acc[(i, t)] = pp if a == 0 else acc[(i, t)] + pp
            ys[(h, x)] = [(acc[(i, 0)] - acc[(i, 2)], acc[(i, 0)] + acc[(i, 1)]) for i in range(no)]

        def combine(h):
            hs = pl.ds(8 * h, 8)
            ab = []
            for i in range(no):
                (r1, i1), (r2, i2) = ys[(h, 0)][i], ys[(h, 1)][i]
                ab.append((r1 + r2, i1 + i2, r1 - r2, i1 - i2))

            def win(cur, prv):
                if prv is None:
                    return cur
                o = []
                for t in range(2):
                    cr, ci, pr_, pi_ = cur[2 * t], cur[2 * t + 1], prv[2 * t], prv[2 * t + 1]
                    o += [cr + pi_, ci - pr_] if sign > 0 else [cr - pi_, ci + pr_]
                return o
            m0 = outs_m[0]
            prv = None if m0 == 0 else [prev_s[(m0 - 1) // 2 + (m0 > 1), rg2, g, t, hs, :] for t in range(4)]
            res = []
            for i in range(no):
                res.append(win(ab[i], prv))
                prv = ab[i]
            outs[h] = res
            ml = outs_m[-1]
            if ml < NU - 1:
                for t in range(4):
                    prev_s[ml // 2 + (ml > 0), rg2, g, t, hs, :] = ab[-1][t]
            if h == 1:
                for i in range(no):
                    for t in range(4):
                        v = jnp.concatenate([outs[0][i][t], outs[1][i][t]], axis=0).astype(bf16)
                        yf_s[outs_m[i], t // 2, g, pl.ds((t % 2) * HL + rg2 * 16, 16), :] = v
            return outs[h][-1][0] + outs[h][-1][1]

        def mk(h):
            def f(pre=None):
                xpart(h, 0, pre)
                xpart(h, 1, None)
                return combine(h)
            return f
        return [mk(0), mk(1)]

    class PRQ:
        def __init__(self, outs_m):
            self.o, self.p = outs_m, 0

        def take(self, k):
            out = [f for p in range(self.p, min(32, self.p + k)) for f in pr_step(self.o, p)]
            self.p = min(32, self.p + k)
            return out

    def lnln(n, layer, half, x):
        rows = pl.ds(n * UL + half * HL, HL)
        x1 = x + _ln(x) * y_s[rows, :]
        x_s[rows, :] = x1
        xn = _ln(x1)
        for g in range(NG):
            xn_s[layer, n, g, pl.ds(half * HL, HL), :] = xn[:, g * 128:(g + 1) * 128].astype(bf16)
        return xn[HL - 8:, 384:512]

    def inv(n, t):
        def fn(deps):
            fi = lhs_cat([fiw[t, 0], fiw[t, 1]], deps)
            ys = [_dot(fi, _b(yfw[n, t, g])) for g in range(NG)]
            y = jnp.concatenate(ys, axis=1)
            y_s[pl.ds(n * UL + t * HL, HL), :] = y
            x = jnp.concatenate([_unp(xw[g, pl.ds(n * HL, HL), :], t) for g in range(NG)], axis=1)
            ptok = lnln(n, 0, t, x)
            return ys[3][HL - 8:], [ptok]
        return fn

    def xn_full(layer, n, deps=()):
        return spread([xnw[layer, n, g] for g in range(NG)], deps)

    def qp(n, layer, c):
        def fn(deps):
            rr = pl.ds(c * QC // 2, QC // 2)
            x = lhs_cat([xnw[layer, n, g, rr, :] for g in range(NG)], [] if RL else deps)
            q = _dot(x, wcat(ww, 0, deps if RL else ()))
            for g in range(NG):
                qb_s[layer, n, g, pl.ds(c * QC, QC), :] = q[:, g * 128:(g + 1) * 128].astype(bf16)
            return q[QC - 8:, 384:512], []
        return fn

    pk_stash = {}

    def ktp(n, layer, c):
        def fn(deps):
            rr = pl.ds(c * KC // 2, KC // 2)
            wk = lhs_cat([wktw[g, rr, :] for g in range(NG)], deps[0::2] if RL else deps)
            if RL and len(deps) > 1:
                p0 = xnw[layer, n, 0]
                p0 = jnp.concatenate([p0[:64], _link(p0[64:], deps[1::2])], axis=0)
                xr = jnp.concatenate([_b(p0)] + [_b(xnw[layer, n, g]) for g in range(1, NG)], axis=1)
            else:
                xr = xn_full(layer, n)
            kt = lax.dot_general(wk, xr, NT, preferred_element_type=f32)
            pk = _phi(kt)
            zz = pk[:, 0:128] + pk[:, 128:256]
            rs = pl.ds(c * KC, KC)
            if n == 0:
                z_s[rs, :] = zz
            else:
                z_s[rs, :] += zz
            pk_stash[(n, layer, c)] = pk.astype(bf16)
            return kt[KC - 8:, 128:256], []
        return fn

    def gp(n, layer, c):
        def fn(deps):
            pk = pk_stash.pop((n, layer, c))
            gg = _dot(pk, xn_full(layer, n, deps))
            rs = pl.ds(c * KC, KC)
            if n == 0:
                g_s[rs, :] = gg
                return gg[KC - 8:, 384:512], []
            new = g_s[rs, :] + gg
            g_s[rs, :] = new
            return gg[KC - 8:, 384:512], [new[KC - 8:, 384:512]]
        return fn

    def qkg_nodes(n, layer):
        nq, nk = UL // QC, D // KC
        qs = [qp(n, layer, c) for c in range(nq)]
        ks = [ktp(n, layer, c) for c in range(nk)]
        gs = [gp(n, layer, c) for c in range(nk)]
        out = []
        for c in range(nk):
            out.append(ks[c])
            if c > 0:
                out.append(gs[c - 1])
            lo, hi = c * nq // nk, (c + 1) * nq // nk
            out += qs[lo:hi]
        out.append(gs[nk - 1])
        return out

    def kg_nodes(n, layer):
        nk = D // KC
        out = []
        for c in range(nk):
            out.append(ktp(n, layer, c))
            if c > 0:
                out.append(gp(n, layer, c - 1))
        out.append(gp(n, layer, nk - 1))
        return out

    def q_nodes(n, layer):
        return [qp(n, layer, c) for c in range(UL // QC)]

    def finalize():
        ri = lax.broadcasted_iota(jnp.int32, (128, 128), 0) >> 4
        ci = lax.broadcasted_iota(jnp.int32, (128, 128), 1) >> 4
        mask = ri == ci
        z = jnp.sum(z_s[...], axis=1, keepdims=True)
        for g in range(NG):
            rs = pl.ds(g * 128, 128)
            zbd_s[g] = jnp.where(mask, z[g * 128:(g + 1) * 128], 0.0).astype(bf16)
            kv = _dot(g_s[rs, :].astype(bf16), _b(ww[8 + g]))
            kv = jnp.where(mask, kv, 0.0).astype(bf16)
            for j in range(NG):
                m_s[j, rs, :] = _dot(kv, _b(wow[j, pl.ds(g * 64, 64), :])).astype(bf16)

    def denp(n, layer, half):
        def fn(deps):
            rr = pl.ds(half * 64, 64)
            tok = None
            for g in range(NG):
                pq = _phi(_b(qbw[layer, n, g, rr, :]).astype(f32))
                den = _dot(pq.astype(bf16), _b(_link(zbw[g], deps))) + 1e-6
                deps = []
                s_s[n, g, pl.ds(half * HL, HL), :] = (pq * pl.reciprocal(den, approx=True)).astype(bf16)
                tok = den[HL - 8:]
            return tok, []
        return fn

    att_stash = {}

    def outp(n, layer, c):
        def fn(deps):
            rr = pl.ds(c * QC // 2, QC // 2)
            s = lhs_cat([sw_[n, g, rr, :] for g in range(NG)], [] if RL else deps)
            a = _dot(s, wcat(mw, 0, deps if RL else ()))
            x2 = x_s[pl.ds(n * UL + c * QC, QC), :] + a
            att_stash.setdefault(n, []).append(x2)
            post = []
            per = HL // QC
            if (c + 1) % per == 0:
                half = c // per
                xh = jnp.concatenate(att_stash[n][half * per:(half + 1) * per], axis=0)
                if layer == 0:
                    post.append(lnln(n, 1, half, xh))
                elif half == 1:
                    xe = jnp.concatenate(att_stash[n][:per], axis=0)
                    pkd = pltpu.pack_elementwise([xe, xh], packed_dtype=bf16)
                    for g in range(NG):
                        ow[g, pl.ds(n * HL, HL), :] = pkd[:, g * 128:(g + 1) * 128]
                    post.append(xh[HL - 8:, 384:512])
                if half == 1:
                    del att_stash[n]
            return a[QC - 8:, 384:512], post
        return fn

    def p2_nodes(n, layer):
        no = UL // QC
        return [denp(n, layer, 0), denp(n, layer, 1)] + [outp(n, layer, c) for c in range(no)]

    def gen_finv():
        for odd in range(2):
            for part in range(2):
                finv_s[odd, part] = _dft_block(odd, part, True, 1.0 / UL).astype(bf16)

    def make_wkt():
        wkt = wcat(ww, 4).T
        for g in range(NG):
            wkt_s[g] = wkt[:, g * 128:(g + 1) * 128]

    def merge(*lists):
        items = []
        for li, l in enumerate(lists):
            lo, hi = 0.0, 1.0
            if isinstance(l, tuple):
                l, lo, hi = l
            for j, x in enumerate(l):
                items.append((lo + (hi - lo) * (j + 0.5) / len(l), li, x))
        items.sort(key=lambda t: (t[0], t[1]))
        return [x for _, _, x in items]

    def run(nodes, *fills):
        assign = [[] for _ in nodes]
        for fillers, i0, i1 in fills:
            nf = len(fillers)
            for j, f in enumerate(fillers):
                assign[i0 + (j * (i1 - i0)) // nf].append(f)
        for fn, fl in zip(nodes, assign):
            node(fn, fl)

    def fufh_nodes(n):
        return [fu(n, (0, 1)), fh(n, (0, 1)), fu(n, (2, 3)), fh(n, (2, 3))]

    def inv_nodes(n):
        return [inv(n, 0), inv(n, 1)]

    cp_sk.start()
    cp_dd.start()
    start(("kv01", 0), ("h", 0), ("kv23", 0))
    for odd in range(2):
        for part in range(2):
            f_s[odd, part] = _dft_block(odd, part, False, 1.0).astype(bf16)
    gen_finv()
    for g in range(NG):
        k_s[g, pl.ds(0, KPAD), :] = jnp.zeros((KPAD, 128), bf16)
    cp_sk.wait()
    cp_dd.wait()
    c_s[pl.ds(0, 4), :] = sk_s[...].astype(f32)
    c_s[pl.ds(4, 1), :] = dd_s[...].astype(f32).reshape(1, D)
    c_s[pl.ds(5, 3), :] = jnp.zeros((3, D), f32)

    p0, p1, p23, p45, p67 = PRQ((0,)), PRQ((1,)), PRQ((2, 3)), PRQ((4, 5)), PRQ((6, 7))
    KG = lambda n: kg_nodes(n, 0)
    Q = lambda n: q_nodes(n, 0)
    FF = fufh_nodes
    INV = inv_nodes
    wait(("kv01", 0))
    start(("xa", 0), ("w", 1))
    run(FF(0)[:1])
    wait(("h", 0))
    start(("kvh", 1))
    run([FF(0)[1], FF(0)[3]])
    wait(("kv23", 0))
    run(FF(0)[2:3])
    wait(("xa", 0), ("w", 1))
    start(("w", 0), ("xb", 1))
    make_wkt()
    for f in p0.take(32):
        f()
    run(INV(0))
    wait(("kvh", 1))
    start(("kvh", 2))
    nd = merge(KG(0)[:4], FF(1)) + KG(0)[4:]
    run(nd, (p1.take(32), 8, 12))
    wait(("w", 0), ("xb", 1), ("kvh", 2))
    start(("kvh", 3), ("xa", 2), ("xb", 3))
    nd = Q(0)[:1] + INV(1) + merge(Q(0)[1:], FF(2)) + KG(1)[:4]
    run(nd)
    wait(("kvh", 3), ("xa", 2), ("xb", 3))
    start(("kvh", 4), ("kvh", 5))
    nd = merge(KG(1)[4:6], FF(3)) + merge(KG(1)[6:], Q(1)) + INV(2) + INV(3)
    run(nd, (p23.take(32), 6, 13))
    wait(("kvh", 4), ("kvh", 5))
    start(("kvh", 6), ("kvh", 7), ("xc", 4), ("xc", 5), ("xc", 6), ("xc", 7))
    nd = merge(FF(4) + FF(5), KG(2)) + merge(KG(3)[:4], Q(2))
    run(nd, (p45.take(PR2A), 16, 24))
    wait(("kvh", 6), ("kvh", 7), ("xc", 4), ("xc", 5), ("xc", 6), ("xc", 7))
    start(("w", 2))
    nd = merge(KG(3)[4:], Q(3), FF(6)[:2]) + INV(4) + INV(5) + merge(FF(6)[2:] + FF(7), KG(4)[:6])
    run(nd, (p45.take(32 - PR2A), 0, 10))
    wait(("w", 2))
    nd = merge(KG(4)[6:], Q(4)) + merge(KG(5)[:6], Q(5)) + INV(6) + KG(5)[6:] + INV(7) \
        + merge(KG(6), Q(6)) + merge(KG(7), Q(7))
    run(nd, (p67.take(32), 0, 16))
    barrier()
    finalize()

    run(p2_nodes(0, 0))
    for n in range(NU):
        if n + 1 < NU:
            run(merge((p2_nodes(n + 1, 0), 0.0, PF), qkg_nodes(n, 1)))
        else:
            run(qkg_nodes(n, 1))
    barrier()
    finalize()

    run(p2_nodes(0, 1)[:2])
    for n in range(NU):
        nxt = p2_nodes(n + 1, 1)[:2] if n + 1 < NU else []
        run(merge(p2_nodes(n, 1)[2:], nxt) if nxt else p2_nodes(n, 1)[2:])
        for g in range(NG):
            out_cp(n, g).start()
    for n in range(NU):
        for g in range(NG):
            out_cp(n, g).wait()


@jax.jit
def pallas_interleave_layers__ssm_conv_h3__linear_attn_block__prompt_kernel(
        A_q, A_k, A_v, A_shift_k, A_ssm_k, A_ssm_D, B_x, B_wqkv, B_wo):
    del B_x
    any_spec = pl.BlockSpec(memory_space=pl.ANY)
    scratch = [
        pltpu.VMEM((NG, S, 128), bf16),
        pltpu.VMEM((NG, S + KPAD, 128), bf16),
        pltpu.VMEM((NG, S, 128), bf16),
        pltpu.VMEM((4, D), bf16),
        pltpu.VMEM((2 * NU, D, 128), bf16),
        pltpu.VMEM((D,), bf16),
        pltpu.VMEM((12, D, 128), bf16),
        pltpu.VMEM((NG, D, 128), bf16),
        pltpu.VMEM((NG, S, 128), bf16),
        pltpu.VMEM((2, 2, HL, HL), bf16),
        pltpu.VMEM((2, 2, HL, HL), bf16),
        pltpu.VMEM((8, D), f32),
        pltpu.VMEM((NG, D, 128), bf16),
        pltpu.VMEM((8, NG, NU, 4, 16, 128), f32),
        pltpu.VMEM((8, NG, NU, 6, 16, 128), f32),
        pltpu.VMEM((NU, 2, NG, UL, 128), bf16),
        pltpu.VMEM((4, 8, NG, 4, 16, 128), f32),
        pltpu.VMEM((S, D), f32),
        pltpu.VMEM((S, D), f32),
        pltpu.VMEM((2, NU, NG, UL, 128), bf16),
        pltpu.VMEM((2, NU, NG, UL, 128), bf16),
        pltpu.VMEM((NU, NG, UL, 128), bf16),
        pltpu.VMEM((D, D), f32),
        pltpu.VMEM((D, 128), f32),
        pltpu.VMEM((NG, 128, 128), bf16),
        pltpu.VMEM((NG, D, 128), bf16),
        pltpu.SemaphoreType.DMA((NU,)),
        pltpu.SemaphoreType.DMA((7,)),
    ]
    out = pl.pallas_call(
        _kernel,
        out_shape=jax.ShapeDtypeStruct((S, D), bf16),
        in_specs=[any_spec] * 8,
        out_specs=any_spec,
        scratch_shapes=scratch,
        compiler_params=pltpu.CompilerParams(vmem_limit_bytes=110 * 1024 * 1024),
    )(A_q.reshape(S, D), A_k.reshape(S, D), A_v.reshape(S, D), A_shift_k.T, A_ssm_k,
      A_ssm_D, B_wqkv, B_wo)
    return out.reshape(1, S, D)
```

```python
import numpy as np
import jax
import jax.numpy as jnp
from jax import lax
import jax.experimental.pallas as pl
import jax.experimental.pallas.tpu as pltpu

S, D = 2048, 512
NU, UL = 8, 256
HL = 128
NG = 4
KPAD = 16
bf16, f32, u32 = jnp.bfloat16, jnp.float32, jnp.uint32
NT = (((1,), (1,)), ((), ()))
QC = 64
KC = 128
PLAG = 4
FWD = 3
PF = 0.5
PR2A = 14
_NEVER = 0x7FC12345


def _cos_pi512(idx):
    t = (256 - jnp.abs(idx)).astype(f32) * (np.pi / 512)
    t2 = t * t
    p = -2.5052108e-08
    for c in (2.7557319e-06, -1.9841270e-04, 8.3333333e-03, -1.6666667e-01, 1.0):
        p = p * t2 + c
    return p * t


def _dft_block(odd, part, transposed, scale):
    r = lax.broadcasted_iota(jnp.int32, (HL, HL), 1 if transposed else 0)
    m = lax.broadcasted_iota(jnp.int32, (HL, HL), 0 if transposed else 1)
    g2 = jnp.where(r < 64, 4 * r + 1, 4 * r - 253)
    idx = (g2 * (2 * m + odd) + (512 - 256 * part)) & 1023
    c = _cos_pi512(idx - 512)
    if scale != 1.0:
        c = c * scale
    return c


def _phi(t):
    return jnp.where(t > 0, t + 1.0, jnp.exp(t)) + 1e-6


def _ln(x):
    m = jnp.mean(x, axis=-1, keepdims=True)
    d = x - m
    v = jnp.mean(d * d, axis=-1, keepdims=True)
    return d * jnp.exp(-0.5 * jnp.log(v + 1e-5))


def _unp(w, i):
    return pltpu.unpack_elementwise(w, index=i, packed_dtype=bf16, unpacked_dtype=f32)


def _dot(a, b):
    return jnp.dot(a, b, preferred_element_type=f32)


def _w(x):
    return pltpu.bitcast(x, u32)


def _b(w):
    return pltpu.bitcast(w, bf16)


def _link(w, deps):
    if not deps:
        return w
    head = w[0:8]
    for d in deps:
        dw = pltpu.bitcast(d, u32)
        head = jnp.where(dw == jnp.uint32(_NEVER), dw, head)
    if w.shape[0] == 8:
        return head
    return jnp.concatenate([head, w[8:]], axis=0)


def _kernel(q_hbm, k_hbm, v_hbm, sk_hbm, h_hbm, dd_hbm, wqkv_hbm, wo_hbm, out_hbm,
            x0_s, k_s, v_s, sk_s, h_s, dd_s, w_s, wo_s, o_s,
            f_s, finv_s, c_s, wkt_s, u_s, hc_s, yf_s, prev_s, y_s, x_s, xn_s, qb_s, s_s,
            g_s, z_s, zbd_s, m_s,
            sem_u, sem_w):
    def lg(g):
        return pl.ds(g * 128, 128)

    def urows(n):
        return pl.ds(n * UL, UL)

    def cp_w(j, sem):
        if j < 12:
            return pltpu.make_async_copy(wqkv_hbm.at[:, lg(j)], w_s.at[j], sem)
        return pltpu.make_async_copy(wo_hbm.at[:, lg(j - 12)], wo_s.at[j - 12], sem)

    def out_cp(n, g):
        return pltpu.make_async_copy(o_s.at[g, urows(n), :], out_hbm.at[urows(n), lg(g)], sem_w.at[0])

    cp_sk = pltpu.make_async_copy(sk_hbm, sk_s, sem_w.at[2])
    cp_dd = pltpu.make_async_copy(dd_hbm, dd_s, sem_w.at[2])

    def copies(tag):
        kind, n = tag
        if kind in ("kvh", "kv01", "kv23", "h"):
            sem = {"kvh": sem_u.at[n], "kv01": sem_u.at[n], "kv23": sem_w.at[5], "h": sem_w.at[6]}[kind]
            gs = {"kvh": (0, 1, 2, 3), "kv01": (0, 1), "kv23": (2, 3), "h": ()}[kind]
            out = []
            for g in gs:
                out.append(pltpu.make_async_copy(k_hbm.at[urows(n), lg(g)],
                                                 k_s.at[g, pl.ds(n * UL + KPAD, UL), :], sem))
                out.append(pltpu.make_async_copy(v_hbm.at[urows(n), lg(g)], v_s.at[g, urows(n), :], sem))
            if kind in ("kvh", "h"):
                out += [pltpu.make_async_copy(h_hbm.at[:, lg(2 * n + t)], h_s.at[2 * n + t], sem)
                        for t in range(2)]
            return out
        if kind in ("xa", "xb", "xc"):
            sem = {"xa": sem_w.at[3], "xb": sem_w.at[4], "xc": sem_w.at[5]}[kind]
            return [pltpu.make_async_copy(q_hbm.at[urows(n), lg(g)], x0_s.at[g, urows(n), :], sem)
                    for g in range(NG)]
        if kind == "w":
            if n == 2:
                return [cp_w(8 + j, sem_w.at[2]) for j in range(8)]
            return [cp_w(4 * n + j, sem_w.at[n]) for j in range(4)]
        raise ValueError(tag)

    def start(*tags):
        for t in tags:
            for c in copies(t):
                c.start()

    def wait(*tags):
        for t in tags:
            for c in copies(t):
                c.wait()

    kw = k_s.bitcast(u32)
    vw = v_s.bitcast(u32)
    xw = x0_s.bitcast(u32)
    hw = h_s.bitcast(u32)
    ww = w_s.bitcast(u32)
    wow = wo_s.bitcast(u32)
    ow = o_s.bitcast(u32)
    fw = f_s.bitcast(u32)
    fiw = finv_s.bitcast(u32)
    wktw = wkt_s.bitcast(u32)
    yfw = yf_s.bitcast(u32)
    xnw = xn_s.bitcast(u32)
    qbw = qb_s.bitcast(u32)
    sw_ = s_s.bitcast(u32)
    zbw = zbd_s.bitcast(u32)
    mw = m_s.bitcast(u32)

    def spread(parts, deps):
        k = len(parts)
        parts = [_link(p, list(deps[i::k])) for i, p in enumerate(parts)]
        return jnp.concatenate([_b(p) for p in parts], axis=1)

    def wcat(ref, j0, deps=()):
        return spread([ref[j0 + j] for j in range(NG)], deps)

    def lhs_cat(parts, deps):
        parts = [_link(parts[0], deps)] + list(parts[1:])
        return jnp.concatenate([_b(p) for p in parts], axis=1) if len(parts) > 1 else _b(parts[0])

    state = {"toks": [], "post": {}}

    def node(fn, fill=()):
        i = len(state["toks"])
        deps = state["post"].pop(i, [])
        pre = state["toks"][i - FWD] if i - FWD >= 0 else None
        for f in fill:
            t = f(pre)
            if t is not None:
                deps.append(t)
        tok, post = fn(deps)
        state["toks"].append(tok)
        if post:
            state["post"].setdefault(i + PLAG, []).extend(post)

    def barrier():
        state["toks"] = []
        state["post"] = {}

    def fwd4(xe, xo, deps):
        fe0 = _b(_link(fw[0, 0], deps))
        er = _dot(fe0, xe)
        pr_ = _dot(_b(fw[1, 0]), xo)
        ei = _dot(_b(fw[0, 1]), xe)
        pi_ = _dot(_b(fw[1, 1]), xo)
        return er, pr_, ei, pi_

    def st_pos(ref, g, n, c, val):
        for r in range(8):
            ref[r, g, n, c] = val[r * 16:(r + 1) * 16]

    def fu(n, gs):
        def fn(deps):
            post = []
            w0 = n * HL
            tok = None
            for g in gs:
                wg = c_s[:, lg(g)]
                W0 = kw[g, pl.ds(w0 + 8, HL), :]
                W1 = kw[g, pl.ds(w0 + 7, HL), :]
                W2 = kw[g, pl.ds(w0 + 6, HL), :]
                e0, o0, e1, o1, o2 = _unp(W0, 0), _unp(W0, 1), _unp(W1, 0), _unp(W1, 1), _unp(W2, 1)
                V = vw[g, pl.ds(w0, HL), :]
                ue = (wg[0:1] * e0 + wg[1:2] * o1 + wg[2:3] * e1 + wg[3:4] * o2) * _unp(V, 0)
                uo = (wg[0:1] * o0 + wg[1:2] * e0 + wg[2:3] * o1 + wg[3:4] * e1) * _unp(V, 1)
                er, pr_, ei, pi_ = fwd4(ue.astype(bf16), uo.astype(bf16), deps)
                deps = []
                st_pos(u_s, g, n, 0, er + pr_)
                st_pos(u_s, g, n, 2, er - pr_)
                st_pos(u_s, g, n, 1, ei + pi_)
                last = ei - pi_
                st_pos(u_s, g, n, 3, last)
                tok = last[HL - 8:]
                post.append(tok)
            return tok, post[:-1]
        return fn

    def fh(n, gs):
        def fn(deps):
            post = []
            tok = None
            for g in gs:
                es, os_ = [], []
                for t in range(2):
                    ht = _b(hw[2 * n + t, pl.ds(g * 64, 64), :]).T
                    W = _w(ht)
                    es.append(_unp(W, 0))
                    os_.append(_unp(W, 1))
                he = jnp.concatenate(es, axis=0).astype(bf16)
                ho = jnp.concatenate(os_, axis=0).astype(bf16)
                er, pr_, ei, pi_ = fwd4(he, ho, deps)
                deps = []
                if n == 0:
                    er = er + c_s[pl.ds(4, 1), lg(g)]
                for x, (c, d) in enumerate(((er + pr_, ei + pi_), (er - pr_, ei - pi_))):
                    st_pos(hc_s, g, n, 3 * x + 0, c)
                    st_pos(hc_s, g, n, 3 * x + 1, d - c)
                    last = c + d
                    st_pos(hc_s, g, n, 3 * x + 2, last)
                tok = last[HL - 8:]
                post.append(tok)
            return tok, post[:-1]
        return fn

    def pr_step(outs_m, p):
        rg2, g = p % 8, p // 8
        sign = 1 if rg2 < 4 else -1
        no = len(outs_m)
        ys = {}
        outs = {}

        def xpart(h, x, pre):
            hs = pl.ds(8 * h, 8)
            acc = {}
            hcache = {}

            def hget(j):
                if j not in hcache:
                    hcache[j] = [hc_s[rg2, g, j, 3 * x + t, hs, :] for t in range(3)]
                return hcache[j]
            for a in range(outs_m[-1] + 1):
                ua = u_s[rg2, g, a, 2 * x, hs, :]
                ub = u_s[rg2, g, a, 2 * x + 1, hs, :]
                if a == 0 and pre is not None:
                    ua = jnp.where(pltpu.bitcast(pre, u32) == jnp.uint32(_NEVER), pre, ua)
                uu = (ua + ub, ua, ub)
                for i in reversed(range(no)):
                    m = outs_m[i]
                    if a > m:
                        continue
                    hh = hget(m - a)
                    for t in range(3):
                        pp = uu[t] * hh[t]
                        acc[(i, t)] = pp if a == 0 else acc[(i, t)] + pp
            ys[(h, x)] = [(acc[(i, 0)] - acc[(i, 2)], acc[(i, 0)] + acc[(i, 1)]) for i in range(no)]

        def combine(h):
            hs = pl.ds(8 * h, 8)
            ab = []
            for i in range(no):
                (r1, i1), (r2, i2) = ys[(h, 0)][i], ys[(h, 1)][i]
                ab.append((r1 + r2, i1 + i2, r1 - r2, i1 - i2))

            def win(cur, prv):
                if prv is None:
                    return cur
                o = []
                for t in range(2):
                    cr, ci, pr_, pi_ = cur[2 * t], cur[2 * t + 1], prv[2 * t], prv[2 * t + 1]
                    o += [cr + pi_, ci - pr_] if sign > 0 else [cr - pi_, ci + pr_]
                return o
            m0 = outs_m[0]
            prv = None if m0 == 0 else [prev_s[(m0 - 1) // 2 + (m0 > 1), rg2, g, t, hs, :] for t in range(4)]
            res = []
            for i in range(no):
                res.append(win(ab[i], prv))
                prv = ab[i]
            outs[h] = res
            ml = outs_m[-1]
            if ml < NU - 1:
                for t in range(4):
                    prev_s[ml // 2 + (ml > 0), rg2, g, t, hs, :] = ab[-1][t]
            if h == 1:
                for i in range(no):
                    for t in range(4):
                        v = jnp.concatenate([outs[0][i][t], outs[1][i][t]], axis=0).astype(bf16)
                        yf_s[outs_m[i], t // 2, g, pl.ds((t % 2) * HL + rg2 * 16, 16), :] = v
            return outs[h][-1][0] + outs[h][-1][1]

        def mk(h):
            def f(pre=None):
                xpart(h, 0, pre)
                xpart(h, 1, None)
                return combine(h)
            return f
        return [mk(0), mk(1)]

    class PRQ:
        def __init__(self, outs_m):
            self.o, self.p = outs_m, 0

        def take(self, k):
            out = [f for p in range(self.p, min(32, self.p + k)) for f in pr_step(self.o, p)]
            self.p = min(32, self.p + k)
            return out

    def lnln(n, layer, half, x):
        rows = pl.ds(n * UL + half * HL, HL)
        x1 = x + _ln(x) * y_s[rows, :]
        x_s[rows, :] = x1
        xn = _ln(x1)
        for g in range(NG):
            xn_s[layer, n, g, pl.ds(half * HL, HL), :] = xn[:, g * 128:(g + 1) * 128].astype(bf16)
        return xn[HL - 8:, 384:512]

    def inv(n, t):
        def fn(deps):
            fi = lhs_cat([fiw[t, 0], fiw[t, 1]], deps)
            ys = [_dot(fi, _b(yfw[n, t, g])) for g in range(NG)]
            y = jnp.concatenate(ys, axis=1)
            y_s[pl.ds(n * UL + t * HL, HL), :] = y
            x = jnp.concatenate([_unp(xw[g, pl.ds(n * HL, HL), :], t) for g in range(NG)], axis=1)
            ptok = lnln(n, 0, t, x)
            return ys[3][HL - 8:], [ptok]
        return fn

    def xn_full(layer, n, deps=()):
        return spread([xnw[layer, n, g] for g in range(NG)], deps)

    def qp(n, layer, c):
        def fn(deps):
            rr = pl.ds(c * QC // 2, QC // 2)
            x = lhs_cat([xnw[layer, n, g, rr, :] for g in range(NG)], [])
            q = _dot(x, wcat(ww, 0, deps))
            for g in range(NG):
                qb_s[layer, n, g, pl.ds(c * QC, QC), :] = q[:, g * 128:(g + 1) * 128].astype(bf16)
            return q[QC - 8:, 384:512], []
        return fn

    pk_stash = {}

    def ktp(n, layer, c):
        def fn(deps):
            rr = pl.ds(c * KC // 2, KC // 2)
            wk = lhs_cat([wktw[g, rr, :] for g in range(NG)], deps[0::2])
            if len(deps) > 1:
                p0 = xnw[layer, n, 0]
                p0 = jnp.concatenate([p0[:64], _link(p0[64:], deps[1::2])], axis=0)
                xr = jnp.concatenate([_b(p0)] + [_b(xnw[layer, n, g]) for g in range(1, NG)], axis=1)
            else:
                xr = xn_full(layer, n)
            kt = lax.dot_general(wk, xr, NT, preferred_element_type=f32)
            pk = _phi(kt)
            zz = pk[:, 0:128] + pk[:, 128:256]
            rs = pl.ds(c * KC, KC)
            if n == 0:
                z_s[rs, :] = zz
            else:
                z_s[rs, :] += zz
            pk_stash[(n, layer, c)] = pk.astype(bf16)
            return kt[KC - 8:, 128:256], []
        return fn

    def gp(n, layer, c):
        def fn(deps):
            pk = pk_stash.pop((n, layer, c))
            gg = _dot(pk, xn_full(layer, n, deps))
            rs = pl.ds(c * KC, KC)
            if n == 0:
                g_s[rs, :] = gg
                return gg[KC - 8:, 384:512], []
            new = g_s[rs, :] + gg
            g_s[rs, :] = new
            return gg[KC - 8:, 384:512], [new[KC - 8:, 384:512]]
        return fn

    def qkg_nodes(n, layer):
        nq, nk = UL // QC, D // KC
        qs = [qp(n, layer, c) for c in range(nq)]
        ks = [ktp(n, layer, c) for c in range(nk)]
        gs = [gp(n, layer, c) for c in range(nk)]
        out = []
        for c in range(nk):
            out.append(ks[c])
            if c > 0:
                out.append(gs[c - 1])
            lo, hi = c * nq // nk, (c + 1) * nq // nk
            out += qs[lo:hi]
        out.append(gs[nk - 1])
        return out

    def kg_nodes(n, layer):
        nk = D // KC
        out = []
        for c in range(nk):
            out.append(ktp(n, layer, c))
            if c > 0:
                out.append(gp(n, layer, c - 1))
        out.append(gp(n, layer, nk - 1))
        return out

    def q_nodes(n, layer):
        return [qp(n, layer, c) for c in range(UL // QC)]

    def finalize():
        ri = lax.broadcasted_iota(jnp.int32, (128, 128), 0) >> 4
        ci = lax.broadcasted_iota(jnp.int32, (128, 128), 1) >> 4
        mask = ri == ci
        z = jnp.sum(z_s[...], axis=1, keepdims=True)
        for g in range(NG):
            rs = pl.ds(g * 128, 128)
            zbd_s[g] = jnp.where(mask, z[g * 128:(g + 1) * 128], 0.0).astype(bf16)
            kv = _dot(g_s[rs, :].astype(bf16), _b(ww[8 + g]))
            kv = jnp.where(mask, kv, 0.0).astype(bf16)
            for j in range(NG):
                m_s[j, rs, :] = _dot(kv, _b(wow[j, pl.ds(g * 64, 64), :])).astype(bf16)

    def denp(n, layer, half):
        def fn(deps):
            rr = pl.ds(half * 64, 64)
            tok = None
            for g in range(NG):
                pq = _phi(_b(qbw[layer, n, g, rr, :]).astype(f32))
                den = _dot(pq.astype(bf16), _b(_link(zbw[g], deps))) + 1e-6
                deps = []
                s_s[n, g, pl.ds(half * HL, HL), :] = (pq * pl.reciprocal(den, approx=True)).astype(bf16)
                tok = den[HL - 8:]
            return tok, []
        return fn

    att_stash = {}

    def out_cp2(n, j, g):
        rows = pl.ds(n * UL + j * 2 * QC, 2 * QC)
        return pltpu.make_async_copy(o_s.at[g, rows, :], out_hbm.at[rows, lg(g)], sem_w.at[0])

    def outp(n, layer, c):
        def fn(deps):
            rr = pl.ds(c * QC // 2, QC // 2)
            s = lhs_cat([sw_[n, g, rr, :] for g in range(NG)], [])
            a = _dot(s, wcat(mw, 0, deps))
            x2 = x_s[pl.ds(n * UL + c * QC, QC), :] + a
            att_stash[(n, c)] = x2
            post = []
            per = HL // QC
            if layer == 0:
                if (c + 1) % per == 0:
                    half = c // per
                    xh = jnp.concatenate([att_stash.pop((n, half * per + j)) for j in range(per)], axis=0)
                    post.append(lnln(n, 1, half, xh))
            elif c >= per:
                j = c - per
                xe = att_stash.pop((n, j))
                xo = att_stash.pop((n, c))
                pkd = pltpu.pack_elementwise([xe, xo], packed_dtype=bf16)
                for g in range(NG):
                    ow[g, pl.ds(n * HL + j * QC, QC), :] = pkd[:, g * 128:(g + 1) * 128]
                if n == NU - 1:
                    for g in range(NG):
                        out_cp2(n, j, g).start()
                post.append(xo[QC - 8:, 384:512])
            return a[QC - 8:, 384:512], post
        return fn

    def p2_nodes(n, layer):
        no = UL // QC
        order = list(range(no))
        if layer == 1:
            order = [c for j in range(no // 2) for c in (j, no // 2 + j)]
        return [denp(n, layer, 0), denp(n, layer, 1)] + [outp(n, layer, c) for c in order]

    def gen_finv():
        for odd in range(2):
            for part in range(2):
                finv_s[odd, part] = _dft_block(odd, part, True, 1.0 / UL).astype(bf16)

    def make_wkt():
        wkt = wcat(ww, 4).T
        for g in range(NG):
            wkt_s[g] = wkt[:, g * 128:(g + 1) * 128]

    def merge(*lists):
        items = []
        for li, l in enumerate(lists):
            lo, hi = 0.0, 1.0
            if isinstance(l, tuple):
                l, lo, hi = l
            for j, x in enumerate(l):
                items.append((lo + (hi - lo) * (j + 0.5) / len(l), li, x))
        items.sort(key=lambda t: (t[0], t[1]))
        return [x for _, _, x in items]

    def run(nodes, *fills):
        assign = [[] for _ in nodes]
        for fillers, i0, i1 in fills:
            nf = len(fillers)
            for j, f in enumerate(fillers):
                assign[i0 + (j * (i1 - i0)) // nf].append(f)
        for fn, fl in zip(nodes, assign):
            node(fn, fl)

    def fufh_nodes(n):
        return [fu(n, (0, 1)), fh(n, (0, 1)), fu(n, (2, 3)), fh(n, (2, 3))]

    def inv_nodes(n):
        return [inv(n, 0), inv(n, 1)]

    cp_sk.start()
    cp_dd.start()
    start(("kv01", 0), ("h", 0), ("kv23", 0))
    for odd in range(2):
        for part in range(2):
            f_s[odd, part] = _dft_block(odd, part, False, 1.0).astype(bf16)
    gen_finv()
    for g in range(NG):
        k_s[g, pl.ds(0, KPAD), :] = jnp.zeros((KPAD, 128), bf16)
    cp_sk.wait()
    cp_dd.wait()
    c_s[pl.ds(0, 4), :] = sk_s[...].astype(f32)
    c_s[pl.ds(4, 1), :] = dd_s[...].astype(f32).reshape(1, D)
    c_s[pl.ds(5, 3), :] = jnp.zeros((3, D), f32)

    p0, p1, p23, p45, p67 = PRQ((0,)), PRQ((1,)), PRQ((2, 3)), PRQ((4, 5)), PRQ((6, 7))
    KG = lambda n: kg_nodes(n, 0)
    Q = lambda n: q_nodes(n, 0)
    FF = fufh_nodes
    INV = inv_nodes
    wait(("kv01", 0))
    start(("xa", 0), ("w", 1))
    run(FF(0)[:1])
    wait(("h", 0))
    start(("kvh", 1))
    run([FF(0)[1], FF(0)[3]])
    wait(("kv23", 0))
    run(FF(0)[2:3])
    wait(("xa", 0), ("w", 1))
    start(("w", 0), ("xb", 1))
    make_wkt()
    for f in p0.take(32):
        f()
    run(INV(0))
    wait(("kvh", 1))
    start(("kvh", 2))
    nd = merge(KG(0)[:4], FF(1)) + KG(0)[4:]
    run(nd, (p1.take(32), 8, 12))
    wait(("w", 0), ("xb", 1), ("kvh", 2))
    start(("kvh", 3), ("xa", 2), ("xb", 3))
    nd = Q(0)[:1] + INV(1) + merge(Q(0)[1:], FF(2)) + KG(1)[:4]
    run(nd)
    wait(("kvh", 3), ("xa", 2), ("xb", 3))
    start(("kvh", 4), ("kvh", 5))
    nd = merge(KG(1)[4:6], FF(3)) + merge(KG(1)[6:], Q(1)[:3]) + INV(2) + Q(1)[3:]
    run(nd, (p23.take(32), 6, 12))
    wait(("kvh", 4), ("kvh", 5))
    start(("kvh", 6), ("kvh", 7), ("xc", 4), ("xc", 5), ("xc", 6), ("xc", 7))
    nd = merge(KG(2), (INV(3), 0.0, 0.3), FF(4) + FF(5)) + merge(KG(3)[:4], Q(2))
    run(nd, (p45.take(PR2A), 18, 26))
    wait(("kvh", 6), ("kvh", 7), ("xc", 4), ("xc", 5), ("xc", 6), ("xc", 7))
    start(("w", 2))
    nd = merge(KG(3)[4:], Q(3), FF(6)[:2]) + INV(4) + INV(5) + merge(KG(4)[:6], FF(6)[2:] + FF(7))
    run(nd, (p45.take(32 - PR2A), 0, 10))
    wait(("w", 2))
    nd = merge(KG(4)[6:], Q(4)) + merge(KG(5), Q(5)[:2]) + INV(6) + INV(7) + Q(5)[2:] \
        + merge(KG(6), Q(6)) + KG(7)
    run(nd, (p67.take(32), 0, 16))
    barrier()
    finalize()

    run(Q(7)[:1] + p2_nodes(0, 0) + Q(7)[1:])
    for n in range(NU):
        if n + 1 < NU:
            run(merge((p2_nodes(n + 1, 0), 0.0, PF), qkg_nodes(n, 1)))
        else:
            run(kg_nodes(n, 1))
    barrier()
    finalize()

    run(q_nodes(NU - 1, 1)[:2] + p2_nodes(0, 1)[:2] + q_nodes(NU - 1, 1)[2:])
    for n in range(NU):
        nxt = p2_nodes(n + 1, 1)[:2] if n + 1 < NU else []
        run(merge(p2_nodes(n, 1)[2:], nxt) if nxt else p2_nodes(n, 1)[2:])
        if n < NU - 1:
            for g in range(NG):
                out_cp(n, g).start()
    for n in range(NU - 1):
        for g in range(NG):
            out_cp(n, g).wait()
    for j in range(UL // QC // 2):
        for g in range(NG):
            out_cp2(NU - 1, j, g).wait()


@jax.jit
def pallas_interleave_layers__ssm_conv_h3__linear_attn_block__prompt_kernel(
        A_q, A_k, A_v, A_shift_k, A_ssm_k, A_ssm_D, B_x, B_wqkv, B_wo):
    del B_x
    any_spec = pl.BlockSpec(memory_space=pl.ANY)
    scratch = [
        pltpu.VMEM((NG, S, 128), bf16),
        pltpu.VMEM((NG, S + KPAD, 128), bf16),
        pltpu.VMEM((NG, S, 128), bf16),
        pltpu.VMEM((4, D), bf16),
        pltpu.VMEM((2 * NU, D, 128), bf16),
        pltpu.VMEM((D,), bf16),
        pltpu.VMEM((12, D, 128), bf16),
        pltpu.VMEM((NG, D, 128), bf16),
        pltpu.VMEM((NG, S, 128), bf16),
        pltpu.VMEM((2, 2, HL, HL), bf16),
        pltpu.VMEM((2, 2, HL, HL), bf16),
        pltpu.VMEM((8, D), f32),
        pltpu.VMEM((NG, D, 128), bf16),
        pltpu.VMEM((8, NG, NU, 4, 16, 128), f32),
        pltpu.VMEM((8, NG, NU, 6, 16, 128), f32),
        pltpu.VMEM((NU, 2, NG, UL, 128), bf16),
        pltpu.VMEM((4, 8, NG, 4, 16, 128), f32),
        pltpu.VMEM((S, D), f32),
        pltpu.VMEM((S, D), f32),
        pltpu.VMEM((2, NU, NG, UL, 128), bf16),
        pltpu.VMEM((2, NU, NG, UL, 128), bf16),
        pltpu.VMEM((NU, NG, UL, 128), bf16),
        pltpu.VMEM((D, D), f32),
        pltpu.VMEM((D, 128), f32),
        pltpu.VMEM((NG, 128, 128), bf16),
        pltpu.VMEM((NG, D, 128), bf16),
        pltpu.SemaphoreType.DMA((NU,)),
        pltpu.SemaphoreType.DMA((7,)),
    ]
    out = pl.pallas_call(
        _kernel,
        out_shape=jax.ShapeDtypeStruct((S, D), bf16),
        in_specs=[any_spec] * 8,
        out_specs=any_spec,
        scratch_shapes=scratch,
        compiler_params=pltpu.CompilerParams(vmem_limit_bytes=110 * 1024 * 1024),
    )(A_q.reshape(S, D), A_k.reshape(S, D), A_v.reshape(S, D), A_shift_k.T, A_ssm_k,
      A_ssm_D, B_wqkv, B_wo)
    return out.reshape(1, S, D)
```

```python
import numpy as np
import jax
import jax.numpy as jnp
from jax import lax
import jax.experimental.pallas as pl
import jax.experimental.pallas.tpu as pltpu

S, D = 2048, 512
NU, UL = 8, 256
HL = 128
NG = 4
KPAD = 16
bf16, f32, u32 = jnp.bfloat16, jnp.float32, jnp.uint32
NT = (((1,), (1,)), ((), ()))
QC = 64
KC = 128
PLAG = 4
FWD = 3
PF = 0.5
PR2A = 14
_NEVER = 0x7FC12345


def _cos_pi512(idx):
    t = (256 - jnp.abs(idx)).astype(f32) * (np.pi / 512)
    t2 = t * t
    p = -2.5052108e-08
    for c in (2.7557319e-06, -1.9841270e-04, 8.3333333e-03, -1.6666667e-01, 1.0):
        p = p * t2 + c
    return p * t


def _dft_block(odd, part, transposed, scale):
    r = lax.broadcasted_iota(jnp.int32, (HL, HL), 1 if transposed else 0)
    m = lax.broadcasted_iota(jnp.int32, (HL, HL), 0 if transposed else 1)
    g2 = jnp.where(r < 64, 4 * r + 1, 4 * r - 253)
    idx = (g2 * (2 * m + odd) + (512 - 256 * part)) & 1023
    c = _cos_pi512(idx - 512)
    if scale != 1.0:
        c = c * scale
    return c


def _phi(t):
    return jnp.where(t > 0, t + 1.0, jnp.exp(t)) + 1e-6


def _ln(x):
    m = jnp.mean(x, axis=-1, keepdims=True)
    d = x - m
    v = jnp.mean(d * d, axis=-1, keepdims=True)
    return d * jnp.exp(-0.5 * jnp.log(v + 1e-5))


def _unp(w, i):
    return pltpu.unpack_elementwise(w, index=i, packed_dtype=bf16, unpacked_dtype=f32)


def _dot(a, b):
    return jnp.dot(a, b, preferred_element_type=f32)


def _w(x):
    return pltpu.bitcast(x, u32)


def _b(w):
    return pltpu.bitcast(w, bf16)


def _link(w, deps):
    if not deps:
        return w
    head = w[0:8]
    for d in deps:
        dw = pltpu.bitcast(d, u32)
        head = jnp.where(dw == jnp.uint32(_NEVER), dw, head)
    if w.shape[0] == 8:
        return head
    return jnp.concatenate([head, w[8:]], axis=0)


def _kernel(q_hbm, k_hbm, v_hbm, sk_hbm, h_hbm, dd_hbm, wqkv_hbm, wo_hbm, out_hbm,
            x0_s, k_s, v_s, sk_s, h_s, dd_s, w_s, wo_s, o_s,
            f_s, finv_s, c_s, wkt_s, u_s, hc_s, yf_s, prev_s, y_s, x_s, xn_s, qb_s, s_s,
            g_s, z_s, zbd_s, m_s,
            sem_u, sem_w):
    def lg(g):
        return pl.ds(g * 128, 128)

    def urows(n):
        return pl.ds(n * UL, UL)

    def cp_w(j, sem):
        if j < 12:
            return pltpu.make_async_copy(wqkv_hbm.at[:, lg(j)], w_s.at[j], sem)
        return pltpu.make_async_copy(wo_hbm.at[:, lg(j - 12)], wo_s.at[j - 12], sem)

    def out_cp(n, g):
        return pltpu.make_async_copy(o_s.at[g, urows(n), :], out_hbm.at[urows(n), lg(g)], sem_w.at[0])

    cp_sk = pltpu.make_async_copy(sk_hbm, sk_s, sem_w.at[2])
    cp_dd = pltpu.make_async_copy(dd_hbm, dd_s, sem_w.at[2])

    def copies(tag):
        kind, n = tag
        if kind in ("kvh", "kv01", "kv23", "h"):
            sem = {"kvh": sem_u.at[n], "kv01": sem_u.at[n], "kv23": sem_w.at[5], "h": sem_w.at[6]}[kind]
            gs = {"kvh": (0, 1, 2, 3), "kv01": (0, 1), "kv23": (2, 3), "h": ()}[kind]
            out = []
            for g in gs:
                out.append(pltpu.make_async_copy(k_hbm.at[urows(n), lg(g)],
                                                 k_s.at[g, pl.ds(n * UL + KPAD, UL), :], sem))
                out.append(pltpu.make_async_copy(v_hbm.at[urows(n), lg(g)], v_s.at[g, urows(n), :], sem))
            if kind in ("kvh", "h"):
                out += [pltpu.make_async_copy(h_hbm.at[:, lg(2 * n + t)], h_s.at[2 * n + t], sem)
                        for t in range(2)]
            return out
        if kind in ("xa", "xb", "xc"):
            sem = {"xa": sem_w.at[3], "xb": sem_w.at[4], "xc": sem_w.at[5]}[kind]
            return [pltpu.make_async_copy(q_hbm.at[urows(n), lg(g)], x0_s.at[g, urows(n), :], sem)
                    for g in range(NG)]
        if kind == "w":
            if n == 2:
                return [cp_w(8 + j, sem_w.at[2]) for j in range(8)]
            return [cp_w(4 * n + j, sem_w.at[n]) for j in range(4)]
        raise ValueError(tag)

    def start(*tags):
        for t in tags:
            for c in copies(t):
                c.start()

    def wait(*tags):
        for t in tags:
            for c in copies(t):
                c.wait()

    kw = k_s.bitcast(u32)
    vw = v_s.bitcast(u32)
    xw = x0_s.bitcast(u32)
    hw = h_s.bitcast(u32)
    ww = w_s.bitcast(u32)
    wow = wo_s.bitcast(u32)
    ow = o_s.bitcast(u32)
    fw = f_s.bitcast(u32)
    fiw = finv_s.bitcast(u32)
    wktw = wkt_s.bitcast(u32)
    yfw = yf_s.bitcast(u32)
    xnw = xn_s.bitcast(u32)
    qbw = qb_s.bitcast(u32)
    sw_ = s_s.bitcast(u32)
    zbw = zbd_s.bitcast(u32)
    mw = m_s.bitcast(u32)

    def spread(parts, deps):
        k = len(parts)
        parts = [_link(p, list(deps[i::k])) for i, p in enumerate(parts)]
        return jnp.concatenate([_b(p) for p in parts], axis=1)

    def wcat(ref, j0, deps=()):
        return spread([ref[j0 + j] for j in range(NG)], deps)

    def lhs_cat(parts, deps):
        parts = [_link(parts[0], deps)] + list(parts[1:])
        return jnp.concatenate([_b(p) for p in parts], axis=1) if len(parts) > 1 else _b(parts[0])

    state = {"toks": [], "post": {}}

    def node(fn, fill=()):
        i = len(state["toks"])
        deps = state["post"].pop(i, [])
        pre = state["toks"][i - FWD] if i - FWD >= 0 else None
        for f in fill:
            t = f(pre)
            if t is not None:
                deps.append(t)
        tok, post = fn(deps)
        state["toks"].append(tok)
        if post:
            state["post"].setdefault(i + PLAG, []).extend(post)

    def barrier():
        state["toks"] = []
        state["post"] = {}

    def fwd4(xe, xo, deps):
        fe0 = _b(_link(fw[0, 0], deps))
        er = _dot(fe0, xe)
        pr_ = _dot(_b(fw[1, 0]), xo)
        ei = _dot(_b(fw[0, 1]), xe)
        pi_ = _dot(_b(fw[1, 1]), xo)
        return er, pr_, ei, pi_

    def st_pos(ref, g, n, c, val):
        for r in range(8):
            ref[r, g, n, c] = val[r * 16:(r + 1) * 16]

    def fu(n, gs):
        def fn(deps):
            post = []
            w0 = n * HL
            tok = None
            for g in gs:
                wg = c_s[:, lg(g)]
                W0 = kw[g, pl.ds(w0 + 8, HL), :]
                W1 = kw[g, pl.ds(w0 + 7, HL), :]
                W2 = kw[g, pl.ds(w0 + 6, HL), :]
                e0, o0, e1, o1, o2 = _unp(W0, 0), _unp(W0, 1), _unp(W1, 0), _unp(W1, 1), _unp(W2, 1)
                V = vw[g, pl.ds(w0, HL), :]
                ue = (wg[0:1] * e0 + wg[1:2] * o1 + wg[2:3] * e1 + wg[3:4] * o2) * _unp(V, 0)
                uo = (wg[0:1] * o0 + wg[1:2] * e0 + wg[2:3] * o1 + wg[3:4] * e1) * _unp(V, 1)
                er, pr_, ei, pi_ = fwd4(ue.astype(bf16), uo.astype(bf16), deps)
                deps = []
                st_pos(u_s, g, n, 0, er + pr_)
                st_pos(u_s, g, n, 2, er - pr_)
                st_pos(u_s, g, n, 1, ei + pi_)
                last = ei - pi_
                st_pos(u_s, g, n, 3, last)
                tok = last[HL - 8:]
                post.append(tok)
            return tok, post[:-1]
        return fn

    def fh(n, gs):
        def fn(deps):
            post = []
            tok = None
            for g in gs:
                es, os_ = [], []
                for t in range(2):
                    ht = _b(hw[2 * n + t, pl.ds(g * 64, 64), :]).T
                    W = _w(ht)
                    es.append(_unp(W, 0))
                    os_.append(_unp(W, 1))
                he = jnp.concatenate(es, axis=0).astype(bf16)
                ho = jnp.concatenate(os_, axis=0).astype(bf16)
                er, pr_, ei, pi_ = fwd4(he, ho, deps)
                deps = []
                if n == 0:
                    er = er + c_s[pl.ds(4, 1), lg(g)]
                for x, (c, d) in enumerate(((er + pr_, ei + pi_), (er - pr_, ei - pi_))):
                    st_pos(hc_s, g, n, 3 * x + 0, c)
                    st_pos(hc_s, g, n, 3 * x + 1, d - c)
                    last = c + d
                    st_pos(hc_s, g, n, 3 * x + 2, last)
                tok = last[HL - 8:]
                post.append(tok)
            return tok, post[:-1]
        return fn

    def pr_step(outs_m, p):
        rg2, g = p % 8, p // 8
        sign = 1 if rg2 < 4 else -1
        no = len(outs_m)
        ys = {}
        outs = {}

        def xpart(h, x, pre):
            hs = pl.ds(8 * h, 8)
            acc = {}
            hcache = {}

            def hget(j):
                if j not in hcache:
                    hcache[j] = [hc_s[rg2, g, j, 3 * x + t, hs, :] for t in range(3)]
                return hcache[j]
            for a in range(outs_m[-1] + 1):
                ua = u_s[rg2, g, a, 2 * x, hs, :]
                ub = u_s[rg2, g, a, 2 * x + 1, hs, :]
                if a == 0 and pre is not None:
                    ua = jnp.where(pltpu.bitcast(pre, u32) == jnp.uint32(_NEVER), pre, ua)
                uu = (ua + ub, ua, ub)
                for i in reversed(range(no)):
                    m = outs_m[i]
                    if a > m:
                        continue
                    hh = hget(m - a)
                    for t in range(3):
                        pp = uu[t] * hh[t]
                        acc[(i, t)] = pp if a == 0 else acc[(i, t)] + pp
            ys[(h, x)] = [(acc[(i, 0)] - acc[(i, 2)], acc[(i, 0)] + acc[(i, 1)]) for i in range(no)]

        def combine(h):
            hs = pl.ds(8 * h, 8)
            ab = []
            for i in range(no):
                (r1, i1), (r2, i2) = ys[(h, 0)][i], ys[(h, 1)][i]
                ab.append((r1 + r2, i1 + i2, r1 - r2, i1 - i2))

            def win(cur, prv):
                if prv is None:
                    return cur
                o = []
                for t in range(2):
                    cr, ci, pr_, pi_ = cur[2 * t], cur[2 * t + 1], prv[2 * t], prv[2 * t + 1]
                    o += [cr + pi_, ci - pr_] if sign > 0 else [cr - pi_, ci + pr_]
                return o
            m0 = outs_m[0]
            prv = None if m0 == 0 else [prev_s[(m0 - 1) // 2 + (m0 > 1), rg2, g, t, hs, :] for t in range(4)]
            res = []
            for i in range(no):
                res.append(win(ab[i], prv))
                prv = ab[i]
            outs[h] = res
            ml = outs_m[-1]
            if ml < NU - 1:
                for t in range(4):
                    prev_s[ml // 2 + (ml > 0), rg2, g, t, hs, :] = ab[-1][t]
            if h == 1:
                for i in range(no):
                    for t in range(4):
                        v = jnp.concatenate([outs[0][i][t], outs[1][i][t]], axis=0).astype(bf16)
                        yf_s[outs_m[i], t // 2, g, pl.ds((t % 2) * HL + rg2 * 16, 16), :] = v
            return outs[h][-1][0] + outs[h][-1][1]

        def mk(h):
            def f(pre=None):
                xpart(h, 0, pre)
                xpart(h, 1, None)
                return combine(h)
            return f
        return [mk(0), mk(1)]

    class PRQ:
        def __init__(self, outs_m):
            self.o, self.p = outs_m, 0

        def take(self, k):
            out = [f for p in range(self.p, min(32, self.p + k)) for f in pr_step(self.o, p)]
            self.p = min(32, self.p + k)
            return out

    def lnln(n, layer, half, x):
        rows = pl.ds(n * UL + half * HL, HL)
        x1 = x + _ln(x) * y_s[rows, :]
        x_s[rows, :] = x1
        xn = _ln(x1)
        for g in range(NG):
            xn_s[layer, n, g, pl.ds(half * HL, HL), :] = xn[:, g * 128:(g + 1) * 128].astype(bf16)
        return xn[HL - 8:, 384:512]

    def inv(n, t):
        def fn(deps):
            fi = lhs_cat([fiw[t, 0], fiw[t, 1]], deps)
            ys = [_dot(fi, _b(yfw[n, t, g])) for g in range(NG)]
            y = jnp.concatenate(ys, axis=1)
            y_s[pl.ds(n * UL + t * HL, HL), :] = y
            x = jnp.concatenate([_unp(xw[g, pl.ds(n * HL, HL), :], t) for g in range(NG)], axis=1)
            ptok = lnln(n, 0, t, x)
            return ys[3][HL - 8:], [ptok]
        return fn

    def xn_full(layer, n, deps=()):
        return spread([xnw[layer, n, g] for g in range(NG)], deps)

    def qp(n, layer, c):
        def fn(deps):
            rr = pl.ds(c * QC // 2, QC // 2)
            x = lhs_cat([xnw[layer, n, g, rr, :] for g in range(NG)], [])
            q = _dot(x, wcat(ww, 0, deps))
            for g in range(NG):
                qb_s[layer, n, g, pl.ds(c * QC, QC), :] = q[:, g * 128:(g + 1) * 128].astype(bf16)
            return q[QC - 8:, 384:512], []
        return fn

    pk_stash = {}

    def ktp(n, layer, c):
        def fn(deps):
            rr = pl.ds(c * KC // 2, KC // 2)
            wk = lhs_cat([wktw[g, rr, :] for g in range(NG)], deps[0::2])
            if len(deps) > 1:
                p0 = xnw[layer, n, 0]
                p0 = jnp.concatenate([p0[:64], _link(p0[64:], deps[1::2])], axis=0)
                xr = jnp.concatenate([_b(p0)] + [_b(xnw[layer, n, g]) for g in range(1, NG)], axis=1)
            else:
                xr = xn_full(layer, n)
            kt = lax.dot_general(wk, xr, NT, preferred_element_type=f32)
            pk = _phi(kt)
            zz = pk[:, 0:128] + pk[:, 128:256]
            rs = pl.ds(c * KC, KC)
            if n == 0:
                z_s[rs, :] = zz
            else:
                z_s[rs, :] += zz
            pk_stash[(n, layer, c)] = pk.astype(bf16)
            return kt[KC - 8:, 128:256], []
        return fn

    def gp(n, layer, c):
        def fn(deps):
            pk = pk_stash.pop((n, layer, c))
            gg = _dot(pk, xn_full(layer, n, deps))
            rs = pl.ds(c * KC, KC)
            if n == 0:
                g_s[rs, :] = gg
                return gg[KC - 8:, 384:512], []
            new = g_s[rs, :] + gg
            g_s[rs, :] = new
            return gg[KC - 8:, 384:512], [new[KC - 8:, 384:512]]
        return fn

    def qkg_nodes(n, layer):
        nq, nk = UL // QC, D // KC
        qs = [qp(n, layer, c) for c in range(nq)]
        ks = [ktp(n, layer, c) for c in range(nk)]
        gs = [gp(n, layer, c) for c in range(nk)]
        out = []
        for c in range(nk):
            out.append(ks[c])
            if c > 0:
                out.append(gs[c - 1])
            lo, hi = c * nq // nk, (c + 1) * nq // nk
            out += qs[lo:hi]
        out.append(gs[nk - 1])
        return out

    def kg_nodes(n, layer):
        nk = D // KC
        out = []
        for c in range(nk):
            out.append(ktp(n, layer, c))
            if c > 0:
                out.append(gp(n, layer, c - 1))
        out.append(gp(n, layer, nk - 1))
        return out

    def q_nodes(n, layer):
        return [qp(n, layer, c) for c in range(UL // QC)]

    def finalize():
        ri = lax.broadcasted_iota(jnp.int32, (128, 128), 0) >> 4
        ci = lax.broadcasted_iota(jnp.int32, (128, 128), 1) >> 4
        mask = ri == ci
        z = jnp.sum(z_s[...], axis=1, keepdims=True)
        for g in range(NG):
            rs = pl.ds(g * 128, 128)
            zbd_s[g] = jnp.where(mask, z[g * 128:(g + 1) * 128], 0.0).astype(bf16)
            kv = _dot(g_s[rs, :].astype(bf16), _b(ww[8 + g]))
            kv = jnp.where(mask, kv, 0.0).astype(bf16)
            for j in range(NG):
                m_s[j, rs, :] = _dot(kv, _b(wow[j, pl.ds(g * 64, 64), :])).astype(bf16)

    def denp(n, layer, half):
        def fn(deps):
            rr = pl.ds(half * 64, 64)
            tok = None
            for g in range(NG):
                pq = _phi(_b(qbw[layer, n, g, rr, :]).astype(f32))
                den = _dot(pq.astype(bf16), _b(_link(zbw[g], deps))) + 1e-6
                deps = []
                s_s[n, g, pl.ds(half * HL, HL), :] = (pq * pl.reciprocal(den, approx=True)).astype(bf16)
                tok = den[HL - 8:]
            return tok, []
        return fn

    att_stash = {}

    def out_cp2(n, j, g):
        rows = pl.ds(n * UL + j * 2 * QC, 2 * QC)
        return pltpu.make_async_copy(o_s.at[g, rows, :], out_hbm.at[rows, lg(g)], sem_w.at[0])

    def outp(n, layer, c):
        def fn(deps):
            rr = pl.ds(c * QC // 2, QC // 2)
            s = lhs_cat([sw_[n, g, rr, :] for g in range(NG)], [])
            a = _dot(s, wcat(mw, 0, deps))
            x2 = x_s[pl.ds(n * UL + c * QC, QC), :] + a
            att_stash[(n, c)] = x2
            post = []
            per = HL // QC
            if layer == 0:
                if (c + 1) % per == 0:
                    half = c // per
                    xh = jnp.concatenate([att_stash.pop((n, half * per + j)) for j in range(per)], axis=0)
                    post.append(lnln(n, 1, half, xh))
            elif c >= per:
                j = c - per
                xe = att_stash.pop((n, j))
                xo = att_stash.pop((n, c))
                pkd = pltpu.pack_elementwise([xe, xo], packed_dtype=bf16)
                for g in range(NG):
                    ow[g, pl.ds(n * HL + j * QC, QC), :] = pkd[:, g * 128:(g + 1) * 128]
                if n == NU - 1:
                    for g in range(NG):
                        out_cp2(n, j, g).start()
                post.append(xo[QC - 8:, 384:512])
            return a[QC - 8:, 384:512], post
        return fn

    def p2_nodes(n, layer):
        no = UL // QC
        order = list(range(no))
        if layer == 1:
            order = [c for j in range(no // 2) for c in (j, no // 2 + j)]
        return [denp(n, layer, 0), denp(n, layer, 1)] + [outp(n, layer, c) for c in order]

    def gen_finv():
        for odd in range(2):
            for part in range(2):
                finv_s[odd, part] = _dft_block(odd, part, True, 1.0 / UL).astype(bf16)

    def make_wkt():
        wkt = wcat(ww, 4).T
        for g in range(NG):
            wkt_s[g] = wkt[:, g * 128:(g + 1) * 128]

    def merge(*lists):
        items = []
        for li, l in enumerate(lists):
            lo, hi = 0.0, 1.0
            if isinstance(l, tuple):
                l, lo, hi = l
            for j, x in enumerate(l):
                items.append((lo + (hi - lo) * (j + 0.5) / len(l), li, x))
        items.sort(key=lambda t: (t[0], t[1]))
        return [x for _, _, x in items]

    def run(nodes, *fills):
        assign = [[] for _ in nodes]
        for fillers, i0, i1 in fills:
            nf = len(fillers)
            for j, f in enumerate(fillers):
                assign[i0 + (j * (i1 - i0)) // nf].append(f)
        for fn, fl in zip(nodes, assign):
            node(fn, fl)

    def fufh_nodes(n):
        return [fu(n, (0, 1)), fh(n, (0, 1)), fu(n, (2, 3)), fh(n, (2, 3))]

    def inv_nodes(n):
        return [inv(n, 0), inv(n, 1)]

    cp_sk.start()
    cp_dd.start()
    start(("kv01", 0), ("h", 0), ("kv23", 0))
    for odd in range(2):
        for part in range(2):
            f_s[odd, part] = _dft_block(odd, part, False, 1.0).astype(bf16)
    gen_finv()
    for g in range(NG):
        k_s[g, pl.ds(0, KPAD), :] = jnp.zeros((KPAD, 128), bf16)
    cp_sk.wait()
    cp_dd.wait()
    c_s[pl.ds(0, 4), :] = sk_s[...].astype(f32)
    c_s[pl.ds(4, 1), :] = dd_s[...].astype(f32).reshape(1, D)
    c_s[pl.ds(5, 3), :] = jnp.zeros((3, D), f32)

    p0, p1, p23, p45, p67 = PRQ((0,)), PRQ((1,)), PRQ((2, 3)), PRQ((4, 5)), PRQ((6, 7))
    KG = lambda n: kg_nodes(n, 0)
    Q = lambda n: q_nodes(n, 0)
    FF = fufh_nodes
    INV = inv_nodes
    wait(("kv01", 0))
    start(("xa", 0), ("w", 1))
    run(FF(0)[:1])
    wait(("h", 0))
    start(("kvh", 1))
    run([FF(0)[1], FF(0)[3]])
    wait(("kv23", 0))
    run(FF(0)[2:3])
    for f in p0.take(32):
        f()
    wait(("xa", 0), ("w", 1))
    start(("w", 0), ("xb", 1))
    make_wkt()
    run(INV(0))
    wait(("kvh", 1))
    start(("kvh", 2))
    nd = merge(KG(0)[:4], FF(1)) + KG(0)[4:]
    run(nd, (p1.take(32), 8, 12))
    wait(("w", 0), ("xb", 1), ("kvh", 2))
    start(("kvh", 3), ("xa", 2), ("xb", 3))
    nd = INV(1) + FF(2) + KG(1)[:4]
    run(nd)
    wait(("kvh", 3), ("xa", 2), ("xb", 3))
    start(("kvh", 4), ("kvh", 5))
    nd = merge(KG(1)[4:6], FF(3)) + merge(KG(1)[6:], Q(0)) + INV(2) + Q(1)[:2]
    run(nd, (p23.take(32), 6, 13))
    wait(("kvh", 4), ("kvh", 5))
    start(("kvh", 6), ("kvh", 7), ("xc", 4), ("xc", 5), ("xc", 6), ("xc", 7))
    nd = merge(KG(2), (INV(3), 0.0, 0.3), FF(4) + FF(5)) + merge(KG(3)[:4], Q(1)[2:], Q(2)[:2])
    run(nd, (p45.take(PR2A), 18, 26))
    wait(("kvh", 6), ("kvh", 7), ("xc", 4), ("xc", 5), ("xc", 6), ("xc", 7))
    start(("w", 2))
    nd = (merge(KG(3)[4:], Q(2)[2:], Q(3), FF(6)[:2]) + INV(4) + INV(5)
          + merge(KG(4)[:6], FF(6)[2:] + FF(7)))
    run(nd, (p45.take(32 - PR2A), 0, 12))
    wait(("w", 2))
    nd = (merge(KG(4)[6:], Q(4)) + merge(KG(5), Q(5)) + INV(6) + INV(7)
          + merge(KG(6), Q(6)) + KG(7))
    run(nd, (p67.take(32), 0, 18))
    barrier()
    finalize()

    run(Q(7)[:1] + p2_nodes(0, 0) + Q(7)[1:])
    for n in range(NU):
        if n + 1 < NU:
            run(merge((p2_nodes(n + 1, 0), 0.0, PF), qkg_nodes(n, 1)))
        else:
            run(kg_nodes(n, 1))
    barrier()
    finalize()

    run(q_nodes(NU - 1, 1)[:2] + p2_nodes(0, 1)[:2] + q_nodes(NU - 1, 1)[2:])
    for n in range(NU):
        nxt = p2_nodes(n + 1, 1)[:2] if n + 1 < NU else []
        run(merge(p2_nodes(n, 1)[2:], nxt) if nxt else p2_nodes(n, 1)[2:])
        if n < NU - 1:
            for g in range(NG):
                out_cp(n, g).start()
    for n in range(NU - 1):
        for g in range(NG):
            out_cp(n, g).wait()
    for j in range(UL // QC // 2):
        for g in range(NG):
            out_cp2(NU - 1, j, g).wait()


@jax.jit
def pallas_interleave_layers__ssm_conv_h3__linear_attn_block__prompt_kernel(
        A_q, A_k, A_v, A_shift_k, A_ssm_k, A_ssm_D, B_x, B_wqkv, B_wo):
    del B_x
    any_spec = pl.BlockSpec(memory_space=pl.ANY)
    scratch = [
        pltpu.VMEM((NG, S, 128), bf16),
        pltpu.VMEM((NG, S + KPAD, 128), bf16),
        pltpu.VMEM((NG, S, 128), bf16),
        pltpu.VMEM((4, D), bf16),
        pltpu.VMEM((2 * NU, D, 128), bf16),
        pltpu.VMEM((D,), bf16),
        pltpu.VMEM((12, D, 128), bf16),
        pltpu.VMEM((NG, D, 128), bf16),
        pltpu.VMEM((NG, S, 128), bf16),
        pltpu.VMEM((2, 2, HL, HL), bf16),
        pltpu.VMEM((2, 2, HL, HL), bf16),
        pltpu.VMEM((8, D), f32),
        pltpu.VMEM((NG, D, 128), bf16),
        pltpu.VMEM((8, NG, NU, 4, 16, 128), f32),
        pltpu.VMEM((8, NG, NU, 6, 16, 128), f32),
        pltpu.VMEM((NU, 2, NG, UL, 128), bf16),
        pltpu.VMEM((4, 8, NG, 4, 16, 128), f32),
        pltpu.VMEM((S, D), f32),
        pltpu.VMEM((S, D), f32),
        pltpu.VMEM((2, NU, NG, UL, 128), bf16),
        pltpu.VMEM((2, NU, NG, UL, 128), bf16),
        pltpu.VMEM((NU, NG, UL, 128), bf16),
        pltpu.VMEM((D, D), f32),
        pltpu.VMEM((D, 128), f32),
        pltpu.VMEM((NG, 128, 128), bf16),
        pltpu.VMEM((NG, D, 128), bf16),
        pltpu.SemaphoreType.DMA((NU,)),
        pltpu.SemaphoreType.DMA((7,)),
    ]
    out = pl.pallas_call(
        _kernel,
        out_shape=jax.ShapeDtypeStruct((S, D), bf16),
        in_specs=[any_spec] * 8,
        out_specs=any_spec,
        scratch_shapes=scratch,
        compiler_params=pltpu.CompilerParams(vmem_limit_bytes=110 * 1024 * 1024),
    )(A_q.reshape(S, D), A_k.reshape(S, D), A_v.reshape(S, D), A_shift_k.T, A_ssm_k,
      A_ssm_D, B_wqkv, B_wo)
    return out.reshape(1, S, D)
```

```python
import numpy as np
import jax
import jax.numpy as jnp
from jax import lax
import jax.experimental.pallas as pl
import jax.experimental.pallas.tpu as pltpu

S, D = 2048, 512
NU, UL = 8, 256
HL = 128
NG = 4
KPAD = 16
bf16, f32, u32 = jnp.bfloat16, jnp.float32, jnp.uint32
NT = (((1,), (1,)), ((), ()))
QC = 64
KC = 128
PLAG = 4
FWD = 3
PF = 0.5
PR2A = 14
_NEVER = 0x7FC12345


def _cos_pi512(idx):
    t = (256 - jnp.abs(idx)).astype(f32) * (np.pi / 512)
    t2 = t * t
    p = -2.5052108e-08
    for c in (2.7557319e-06, -1.9841270e-04, 8.3333333e-03, -1.6666667e-01, 1.0):
        p = p * t2 + c
    return p * t


def _dft_block(odd, part, transposed, scale):
    r = lax.broadcasted_iota(jnp.int32, (HL, HL), 1 if transposed else 0)
    m = lax.broadcasted_iota(jnp.int32, (HL, HL), 0 if transposed else 1)
    g2 = jnp.where(r < 64, 4 * r + 1, 4 * r - 253)
    idx = (g2 * (2 * m + odd) + (512 - 256 * part)) & 1023
    c = _cos_pi512(idx - 512)
    if scale != 1.0:
        c = c * scale
    return c


def _phi(t):
    return jnp.where(t > 0, t + 1.0, jnp.exp(t)) + 1e-6


def _ln(x):
    m = jnp.mean(x, axis=-1, keepdims=True)
    d = x - m
    v = jnp.mean(d * d, axis=-1, keepdims=True)
    return d * jnp.exp(-0.5 * jnp.log(v + 1e-5))


def _unp(w, i):
    return pltpu.unpack_elementwise(w, index=i, packed_dtype=bf16, unpacked_dtype=f32)


def _dot(a, b):
    return jnp.dot(a, b, preferred_element_type=f32)


def _w(x):
    return pltpu.bitcast(x, u32)


def _b(w):
    return pltpu.bitcast(w, bf16)


def _link(w, deps):
    if not deps:
        return w
    head = w[0:8]
    for d in deps:
        dw = pltpu.bitcast(d, u32)
        head = jnp.where(dw == jnp.uint32(_NEVER), dw, head)
    if w.shape[0] == 8:
        return head
    return jnp.concatenate([head, w[8:]], axis=0)


def _kernel(q_hbm, k_hbm, v_hbm, sk_hbm, h_hbm, dd_hbm, wqkv_hbm, wo_hbm, out_hbm,
            x0_s, k_s, v_s, sk_s, h_s, dd_s, w_s, wo_s, o_s,
            f_s, finv_s, c_s, wkt_s, u_s, hc_s, yf_s, prev_s, y_s, x_s, xn_s, qb_s, s_s,
            g_s, z_s, zbd_s, m_s,
            sem_u, sem_w):
    def lg(g):
        return pl.ds(g * 128, 128)

    def urows(n):
        return pl.ds(n * UL, UL)

    def cp_w(j, sem):
        if j < 12:
            return pltpu.make_async_copy(wqkv_hbm.at[:, lg(j)], w_s.at[j], sem)
        return pltpu.make_async_copy(wo_hbm.at[:, lg(j - 12)], wo_s.at[j - 12], sem)

    def out_cp(n, g):
        return pltpu.make_async_copy(o_s.at[g, urows(n), :], out_hbm.at[urows(n), lg(g)], sem_w.at[0])

    cp_sk = pltpu.make_async_copy(sk_hbm, sk_s, sem_w.at[2])
    cp_dd = pltpu.make_async_copy(dd_hbm, dd_s, sem_w.at[2])

    def copies(tag):
        kind, n = tag
        if kind in ("kvh", "kv01", "kv23", "h"):
            sem = {"kvh": sem_u.at[n], "kv01": sem_u.at[n], "kv23": sem_w.at[5], "h": sem_w.at[6]}[kind]
            gs = {"kvh": (0, 1, 2, 3), "kv01": (0, 1), "kv23": (2, 3), "h": ()}[kind]
            out = []
            for g in gs:
                out.append(pltpu.make_async_copy(k_hbm.at[urows(n), lg(g)],
                                                 k_s.at[g, pl.ds(n * UL + KPAD, UL), :], sem))
                out.append(pltpu.make_async_copy(v_hbm.at[urows(n), lg(g)], v_s.at[g, urows(n), :], sem))
            if kind in ("kvh", "h"):
                out += [pltpu.make_async_copy(h_hbm.at[:, lg(2 * n + t)], h_s.at[2 * n + t], sem)
                        for t in range(2)]
            return out
        if kind in ("xa", "xb", "xc"):
            sem = {"xa": sem_w.at[3], "xb": sem_w.at[4], "xc": sem_w.at[5]}[kind]
            return [pltpu.make_async_copy(q_hbm.at[urows(n), lg(g)], x0_s.at[g, urows(n), :], sem)
                    for g in range(NG)]
        if kind == "w":
            if n == 2:
                return [cp_w(8 + j, sem_w.at[2]) for j in range(8)]
            return [cp_w(4 * n + j, sem_w.at[n]) for j in range(4)]
        raise ValueError(tag)

    def start(*tags):
        for t in tags:
            for c in copies(t):
                c.start()

    def wait(*tags):
        for t in tags:
            for c in copies(t):
                c.wait()

    kw = k_s.bitcast(u32)
    vw = v_s.bitcast(u32)
    xw = x0_s.bitcast(u32)
    hw = h_s.bitcast(u32)
    ww = w_s.bitcast(u32)
    wow = wo_s.bitcast(u32)
    ow = o_s.bitcast(u32)
    fw = f_s.bitcast(u32)
    fiw = finv_s.bitcast(u32)
    wktw = wkt_s.bitcast(u32)
    yfw = yf_s.bitcast(u32)
    xnw = xn_s.bitcast(u32)
    qbw = qb_s.bitcast(u32)
    sw_ = s_s.bitcast(u32)
    zbw = zbd_s.bitcast(u32)
    mw = m_s.bitcast(u32)

    def spread(parts, deps):
        k = len(parts)
        parts = [_link(p, list(deps[i::k])) for i, p in enumerate(parts)]
        return jnp.concatenate([_b(p) for p in parts], axis=1)

    def wcat(ref, j0, deps=()):
        return spread([ref[j0 + j] for j in range(NG)], deps)

    def lhs_cat(parts, deps):
        parts = [_link(parts[0], deps)] + list(parts[1:])
        return jnp.concatenate([_b(p) for p in parts], axis=1) if len(parts) > 1 else _b(parts[0])

    state = {"toks": [], "post": {}}

    def node(fn, fill=()):
        i = len(state["toks"])
        deps = state["post"].pop(i, [])
        pre = state["toks"][i - FWD] if i - FWD >= 0 else None
        for f in fill:
            t = f(pre)
            if t is not None:
                deps.append(t)
        tok, post = fn(deps)
        state["toks"].append(tok)
        if post:
            state["post"].setdefault(i + PLAG, []).extend(post)

    def barrier():
        state["toks"] = []
        state["post"] = {}

    def fwd4(xe, xo, deps):
        fe0 = _b(_link(fw[0, 0], deps))
        er = _dot(fe0, xe)
        pr_ = _dot(_b(fw[1, 0]), xo)
        ei = _dot(_b(fw[0, 1]), xe)
        pi_ = _dot(_b(fw[1, 1]), xo)
        return er, pr_, ei, pi_

    def st_pos(ref, g, n, c, val):
        for r in range(8):
            ref[r, g, n, c] = val[r * 16:(r + 1) * 16]

    def fu(n, gs):
        def fn(deps):
            post = []
            w0 = n * HL
            tok = None
            for g in gs:
                wg = c_s[:, lg(g)]
                W0 = kw[g, pl.ds(w0 + 8, HL), :]
                W1 = kw[g, pl.ds(w0 + 7, HL), :]
                W2 = kw[g, pl.ds(w0 + 6, HL), :]
                e0, o0, e1, o1, o2 = _unp(W0, 0), _unp(W0, 1), _unp(W1, 0), _unp(W1, 1), _unp(W2, 1)
                V = vw[g, pl.ds(w0, HL), :]
                ue = (wg[0:1] * e0 + wg[1:2] * o1 + wg[2:3] * e1 + wg[3:4] * o2) * _unp(V, 0)
                uo = (wg[0:1] * o0 + wg[1:2] * e0 + wg[2:3] * o1 + wg[3:4] * e1) * _unp(V, 1)
                er, pr_, ei, pi_ = fwd4(ue.astype(bf16), uo.astype(bf16), deps)
                deps = []
                st_pos(u_s, g, n, 0, er + pr_)
                st_pos(u_s, g, n, 2, er - pr_)
                st_pos(u_s, g, n, 1, ei + pi_)
                last = ei - pi_
                st_pos(u_s, g, n, 3, last)
                tok = last[HL - 8:]
                post.append(tok)
            return tok, post[:-1]
        return fn

    def fh(n, gs):
        def fn(deps):
            post = []
            tok = None
            for g in gs:
                es, os_ = [], []
                for t in range(2):
                    ht = _b(hw[2 * n + t, pl.ds(g * 64, 64), :]).T
                    W = _w(ht)
                    es.append(_unp(W, 0))
                    os_.append(_unp(W, 1))
                he = jnp.concatenate(es, axis=0).astype(bf16)
                ho = jnp.concatenate(os_, axis=0).astype(bf16)
                er, pr_, ei, pi_ = fwd4(he, ho, deps)
                deps = []
                if n == 0:
                    er = er + c_s[pl.ds(4, 1), lg(g)]
                for x, (c, d) in enumerate(((er + pr_, ei + pi_), (er - pr_, ei - pi_))):
                    st_pos(hc_s, g, n, 3 * x + 0, c)
                    st_pos(hc_s, g, n, 3 * x + 1, d - c)
                    last = c + d
                    st_pos(hc_s, g, n, 3 * x + 2, last)
                tok = last[HL - 8:]
                post.append(tok)
            return tok, post[:-1]
        return fn

    def pr_step(outs_m, p):
        rg2, g = p % 8, p // 8
        sign = 1 if rg2 < 4 else -1
        no = len(outs_m)
        ys = {}
        outs = {}

        def xpart(h, x, pre):
            hs = pl.ds(8 * h, 8)
            acc = {}
            hcache = {}

            def hget(j):
                if j not in hcache:
                    hcache[j] = [hc_s[rg2, g, j, 3 * x + t, hs, :] for t in range(3)]
                return hcache[j]
            for a in range(outs_m[-1] + 1):
                ua = u_s[rg2, g, a, 2 * x, hs, :]
                ub = u_s[rg2, g, a, 2 * x + 1, hs, :]
                if a == 0 and pre is not None:
                    ua = jnp.where(pltpu.bitcast(pre, u32) == jnp.uint32(_NEVER), pre, ua)
                uu = (ua + ub, ua, ub)
                for i in reversed(range(no)):
                    m = outs_m[i]
                    if a > m:
                        continue
                    hh = hget(m - a)
                    for t in range(3):
                        pp = uu[t] * hh[t]
                        acc[(i, t)] = pp if a == 0 else acc[(i, t)] + pp
            ys[(h, x)] = [(acc[(i, 0)] - acc[(i, 2)], acc[(i, 0)] + acc[(i, 1)]) for i in range(no)]

        def combine(h):
            hs = pl.ds(8 * h, 8)
            ab = []
            for i in range(no):
                (r1, i1), (r2, i2) = ys[(h, 0)][i], ys[(h, 1)][i]
                ab.append((r1 + r2, i1 + i2, r1 - r2, i1 - i2))

            def win(cur, prv):
                if prv is None:
                    return cur
                o = []
                for t in range(2):
                    cr, ci, pr_, pi_ = cur[2 * t], cur[2 * t + 1], prv[2 * t], prv[2 * t + 1]
                    o += [cr + pi_, ci - pr_] if sign > 0 else [cr - pi_, ci + pr_]
                return o
            m0 = outs_m[0]
            prv = None if m0 == 0 else [prev_s[(m0 - 1) // 2 + (m0 > 1), rg2, g, t, hs, :] for t in range(4)]
            res = []
            for i in range(no):
                res.append(win(ab[i], prv))
                prv = ab[i]
            outs[h] = res
            ml = outs_m[-1]
            if ml < NU - 1:
                for t in range(4):
                    prev_s[ml // 2 + (ml > 0), rg2, g, t, hs, :] = ab[-1][t]
            if h == 1:
                for i in range(no):
                    for t in range(4):
                        v = jnp.concatenate([outs[0][i][t], outs[1][i][t]], axis=0).astype(bf16)
                        yf_s[outs_m[i], t // 2, g, pl.ds((t % 2) * HL + rg2 * 16, 16), :] = v
            return outs[h][-1][0] + outs[h][-1][1]

        def mk(h):
            def f(pre=None):
                xpart(h, 0, pre)
                xpart(h, 1, None)
                return combine(h)
            return f
        return [mk(0), mk(1)]

    class PRQ:
        def __init__(self, outs_m):
            self.o, self.p = outs_m, 0

        def take(self, k):
            out = [f for p in range(self.p, min(32, self.p + k)) for f in pr_step(self.o, p)]
            self.p = min(32, self.p + k)
            return out

    def lnln(n, layer, half, x):
        rows = pl.ds(n * UL + half * HL, HL)
        x1 = x + _ln(x) * y_s[rows, :]
        x_s[rows, :] = x1
        xn = _ln(x1)
        for g in range(NG):
            xn_s[layer, n, g, pl.ds(half * HL, HL), :] = xn[:, g * 128:(g + 1) * 128].astype(bf16)
        return xn[HL - 8:, 384:512]

    def inv(n, t):
        def fn(deps):
            fi = lhs_cat([fiw[t, 0], fiw[t, 1]], deps)
            ys = [_dot(fi, _b(yfw[n, t, g])) for g in range(NG)]
            y = jnp.concatenate(ys, axis=1)
            y_s[pl.ds(n * UL + t * HL, HL), :] = y
            x = jnp.concatenate([_unp(xw[g, pl.ds(n * HL, HL), :], t) for g in range(NG)], axis=1)
            ptok = lnln(n, 0, t, x)
            return ys[3][HL - 8:], [ptok]
        return fn

    def xn_full(layer, n, deps=()):
        return spread([xnw[layer, n, g] for g in range(NG)], deps)

    def qp(n, layer, c):
        def fn(deps):
            rr = pl.ds(c * QC // 2, QC // 2)
            x = lhs_cat([xnw[layer, n, g, rr, :] for g in range(NG)], [])
            q = _dot(x, wcat(ww, 0, deps))
            for g in range(NG):
                qb_s[layer, n, g, pl.ds(c * QC, QC), :] = q[:, g * 128:(g + 1) * 128].astype(bf16)
            return q[QC - 8:, 384:512], []
        return fn

    pk_stash = {}

    def ktp(n, layer, c):
        def fn(deps):
            rr = pl.ds(c * KC // 2, KC // 2)
            wk = lhs_cat([wktw[g, rr, :] for g in range(NG)], deps[0::2])
            if len(deps) > 1:
                p0 = xnw[layer, n, 0]
                p0 = jnp.concatenate([p0[:64], _link(p0[64:], deps[1::2])], axis=0)
                xr = jnp.concatenate([_b(p0)] + [_b(xnw[layer, n, g]) for g in range(1, NG)], axis=1)
            else:
                xr = xn_full(layer, n)
            kt = lax.dot_general(wk, xr, NT, preferred_element_type=f32)
            pk = _phi(kt)
            zz = pk[:, 0:128] + pk[:, 128:256]
            rs = pl.ds(c * KC, KC)
            if n == 0:
                z_s[rs, :] = zz
            else:
                z_s[rs, :] += zz
            pk_stash[(n, layer, c)] = pk.astype(bf16)
            return kt[KC - 8:, 128:256], []
        return fn

    def gp(n, layer, c):
        def fn(deps):
            pk = pk_stash.pop((n, layer, c))
            gg = _dot(pk, xn_full(layer, n, deps))
            rs = pl.ds(c * KC, KC)
            if n == 0:
                g_s[rs, :] = gg
                return gg[KC - 8:, 384:512], []
            new = g_s[rs, :] + gg
            g_s[rs, :] = new
            return gg[KC - 8:, 384:512], [new[KC - 8:, 384:512]]
        return fn

    def qkg_nodes(n, layer):
        nq, nk = UL // QC, D // KC
        qs = [qp(n, layer, c) for c in range(nq)]
        ks = [ktp(n, layer, c) for c in range(nk)]
        gs = [gp(n, layer, c) for c in range(nk)]
        out = []
        for c in range(nk):
            out.append(ks[c])
            if c > 0:
                out.append(gs[c - 1])
            lo, hi = c * nq // nk, (c + 1) * nq // nk
            out += qs[lo:hi]
        out.append(gs[nk - 1])
        return out

    def kg_nodes(n, layer):
        nk = D // KC
        out = []
        for c in range(nk):
            out.append(ktp(n, layer, c))
            if c > 0:
                out.append(gp(n, layer, c - 1))
        out.append(gp(n, layer, nk - 1))
        return out

    def q_nodes(n, layer):
        return [qp(n, layer, c) for c in range(UL // QC)]

    def finalize():
        ri = lax.broadcasted_iota(jnp.int32, (128, 128), 0) >> 4
        ci = lax.broadcasted_iota(jnp.int32, (128, 128), 1) >> 4
        mask = ri == ci
        z = jnp.sum(z_s[...], axis=1, keepdims=True)
        for g in range(NG):
            rs = pl.ds(g * 128, 128)
            zbd_s[g] = jnp.where(mask, z[g * 128:(g + 1) * 128], 0.0).astype(bf16)
            kv = _dot(g_s[rs, :].astype(bf16), _b(ww[8 + g]))
            kv = jnp.where(mask, kv, 0.0).astype(bf16)
            for j in range(NG):
                m_s[j, rs, :] = _dot(kv, _b(wow[j, pl.ds(g * 64, 64), :])).astype(bf16)

    def denp(n, layer, half):
        def fn(deps):
            rr = pl.ds(half * 64, 64)
            tok = None
            for g in range(NG):
                pq = _phi(_b(qbw[layer, n, g, rr, :]).astype(f32))
                den = _dot(pq.astype(bf16), _b(_link(zbw[g], deps))) + 1e-6
                deps = []
                s_s[n, g, pl.ds(half * HL, HL), :] = (pq * pl.reciprocal(den, approx=True)).astype(bf16)
                tok = den[HL - 8:]
            return tok, []
        return fn

    att_stash = {}

    def out_cp2(n, j, g):
        rows = pl.ds(n * UL + j * 2 * QC, 2 * QC)
        return pltpu.make_async_copy(o_s.at[g, rows, :], out_hbm.at[rows, lg(g)], sem_w.at[0])

    def outp(n, layer, c):
        def fn(deps):
            rr = pl.ds(c * QC // 2, QC // 2)
            s = lhs_cat([sw_[n, g, rr, :] for g in range(NG)], [])
            a = _dot(s, wcat(mw, 0, deps))
            x2 = x_s[pl.ds(n * UL + c * QC, QC), :] + a
            att_stash[(n, c)] = x2
            post = []
            per = HL // QC
            if layer == 0:
                if (c + 1) % per == 0:
                    half = c // per
                    xh = jnp.concatenate([att_stash.pop((n, half * per + j)) for j in range(per)], axis=0)
                    post.append(lnln(n, 1, half, xh))
            elif c >= per:
                j = c - per
                xe = att_stash.pop((n, j))
                xo = att_stash.pop((n, c))
                pkd = pltpu.pack_elementwise([xe, xo], packed_dtype=bf16)
                for g in range(NG):
                    ow[g, pl.ds(n * HL + j * QC, QC), :] = pkd[:, g * 128:(g + 1) * 128]
                if n == NU - 1:
                    for g in range(NG):
                        out_cp2(n, j, g).start()
                post.append(xo[QC - 8:, 384:512])
            return a[QC - 8:, 384:512], post
        return fn

    def p2_nodes(n, layer):
        no = UL // QC
        order = list(range(no))
        if layer == 1:
            order = [c for j in range(no // 2) for c in (j, no // 2 + j)]
        return [denp(n, layer, 0), denp(n, layer, 1)] + [outp(n, layer, c) for c in order]

    def gen_finv():
        for odd in range(2):
            for part in range(2):
                finv_s[odd, part] = _dft_block(odd, part, True, 1.0 / UL).astype(bf16)

    def make_wkt():
        wkt = wcat(ww, 4).T
        for g in range(NG):
            wkt_s[g] = wkt[:, g * 128:(g + 1) * 128]

    def merge(*lists):
        items = []
        for li, l in enumerate(lists):
            lo, hi = 0.0, 1.0
            if isinstance(l, tuple):
                l, lo, hi = l
            for j, x in enumerate(l):
                items.append((lo + (hi - lo) * (j + 0.5) / len(l), li, x))
        items.sort(key=lambda t: (t[0], t[1]))
        return [x for _, _, x in items]

    def run(nodes, *fills):
        assign = [[] for _ in nodes]
        for fillers, i0, i1 in fills:
            nf = len(fillers)
            for j, f in enumerate(fillers):
                assign[i0 + (j * (i1 - i0)) // nf].append(f)
        for fn, fl in zip(nodes, assign):
            node(fn, fl)

    def fufh_nodes(n):
        return [fu(n, (0, 1)), fh(n, (0, 1)), fu(n, (2, 3)), fh(n, (2, 3))]

    def inv_nodes(n):
        return [inv(n, 0), inv(n, 1)]

    cp_sk.start()
    cp_dd.start()
    start(("h", 0), ("kv01", 0), ("kv23", 0))
    for odd in range(2):
        for part in range(2):
            f_s[odd, part] = _dft_block(odd, part, False, 1.0).astype(bf16)
    gen_finv()
    for g in range(NG):
        k_s[g, pl.ds(0, KPAD), :] = jnp.zeros((KPAD, 128), bf16)
    cp_sk.wait()
    cp_dd.wait()
    c_s[pl.ds(0, 4), :] = sk_s[...].astype(f32)
    c_s[pl.ds(4, 1), :] = dd_s[...].astype(f32).reshape(1, D)
    c_s[pl.ds(5, 3), :] = jnp.zeros((3, D), f32)

    p0, p1, p23, p45, p67 = PRQ((0,)), PRQ((1,)), PRQ((2, 3)), PRQ((4, 5)), PRQ((6, 7))
    KG = lambda n: kg_nodes(n, 0)
    Q = lambda n: q_nodes(n, 0)
    FF = fufh_nodes
    INV = inv_nodes
    wait(("h", 0))
    start(("xa", 0), ("w", 1))
    run([FF(0)[1], FF(0)[3]])
    wait(("kv01", 0), ("kv23", 0))
    start(("kvh", 1))
    run([FF(0)[0], FF(0)[2]])
    for f in p0.take(32):
        f()
    wait(("xa", 0), ("w", 1))
    start(("xb", 1), ("kvh", 2))
    make_wkt()
    run(INV(0))
    wait(("kvh", 1))
    start(("kvh", 3), ("w", 0))
    nd = merge(KG(0)[:4], FF(1)) + KG(0)[4:]
    run(nd, (p1.take(32), 8, 12))
    wait(("xb", 1), ("kvh", 2))
    start(("xa", 2), ("xb", 3), ("kvh", 4))
    nd = INV(1) + FF(2) + KG(1)[:4]
    run(nd)
    wait(("kvh", 3), ("w", 0), ("xa", 2), ("xb", 3))
    start(("kvh", 5), ("kvh", 6))
    nd = merge(KG(1)[4:6], FF(3)) + merge(KG(1)[6:], Q(0)) + INV(2) + Q(1)[:2]
    run(nd, (p23.take(32), 6, 13))
    wait(("kvh", 4), ("kvh", 5))
    start(("kvh", 7), ("xc", 4), ("xc", 5), ("xc", 6), ("xc", 7))
    nd = merge(KG(2), (INV(3), 0.0, 0.3), FF(4) + FF(5)) + merge(KG(3)[:4], Q(1)[2:], Q(2)[:2])
    run(nd, (p45.take(PR2A), 18, 26))
    wait(("kvh", 6), ("kvh", 7), ("xc", 4), ("xc", 5), ("xc", 6), ("xc", 7))
    start(("w", 2))
    nd = (merge(KG(3)[4:], Q(2)[2:], Q(3), FF(6)[:2]) + INV(4) + INV(5)
          + merge(KG(4)[:6], FF(6)[2:] + FF(7)))
    run(nd, (p45.take(32 - PR2A), 0, 12))
    wait(("w", 2))
    nd = (merge(KG(4)[6:], Q(4)) + merge(KG(5), Q(5)) + INV(6) + INV(7)
          + merge(KG(6), Q(6)) + KG(7))
    run(nd, (p67.take(32), 0, 18))
    barrier()
    finalize()

    run(Q(7)[:1] + p2_nodes(0, 0) + Q(7)[1:])
    for n in range(NU):
        if n + 1 < NU:
            run(merge((p2_nodes(n + 1, 0), 0.0, PF), qkg_nodes(n, 1)))
        else:
            run(kg_nodes(n, 1))
    barrier()
    finalize()

    run(q_nodes(NU - 1, 1)[:2] + p2_nodes(0, 1)[:2] + q_nodes(NU - 1, 1)[2:])
    for n in range(NU):
        nxt = p2_nodes(n + 1, 1)[:2] if n + 1 < NU else []
        run(merge(p2_nodes(n, 1)[2:], nxt) if nxt else p2_nodes(n, 1)[2:])
        if n < NU - 1:
            for g in range(NG):
                out_cp(n, g).start()
    for n in range(NU - 1):
        for g in range(NG):
            out_cp(n, g).wait()
    for j in range(UL // QC // 2):
        for g in range(NG):
            out_cp2(NU - 1, j, g).wait()


@jax.jit
def pallas_interleave_layers__ssm_conv_h3__linear_attn_block__prompt_kernel(
        A_q, A_k, A_v, A_shift_k, A_ssm_k, A_ssm_D, B_x, B_wqkv, B_wo):
    del B_x
    any_spec = pl.BlockSpec(memory_space=pl.ANY)
    scratch = [
        pltpu.VMEM((NG, S, 128), bf16),
        pltpu.VMEM((NG, S + KPAD, 128), bf16),
        pltpu.VMEM((NG, S, 128), bf16),
        pltpu.VMEM((4, D), bf16),
        pltpu.VMEM((2 * NU, D, 128), bf16),
        pltpu.VMEM((D,), bf16),
        pltpu.VMEM((12, D, 128), bf16),
        pltpu.VMEM((NG, D, 128), bf16),
        pltpu.VMEM((NG, S, 128), bf16),
        pltpu.VMEM((2, 2, HL, HL), bf16),
        pltpu.VMEM((2, 2, HL, HL), bf16),
        pltpu.VMEM((8, D), f32),
        pltpu.VMEM((NG, D, 128), bf16),
        pltpu.VMEM((8, NG, NU, 4, 16, 128), f32),
        pltpu.VMEM((8, NG, NU, 6, 16, 128), f32),
        pltpu.VMEM((NU, 2, NG, UL, 128), bf16),
        pltpu.VMEM((4, 8, NG, 4, 16, 128), f32),
        pltpu.VMEM((S, D), f32),
        pltpu.VMEM((S, D), f32),
        pltpu.VMEM((2, NU, NG, UL, 128), bf16),
        pltpu.VMEM((2, NU, NG, UL, 128), bf16),
        pltpu.VMEM((NU, NG, UL, 128), bf16),
        pltpu.VMEM((D, D), f32),
        pltpu.VMEM((D, 128), f32),
        pltpu.VMEM((NG, 128, 128), bf16),
        pltpu.VMEM((NG, D, 128), bf16),
        pltpu.SemaphoreType.DMA((NU,)),
        pltpu.SemaphoreType.DMA((7,)),
    ]
    out = pl.pallas_call(
        _kernel,
        out_shape=jax.ShapeDtypeStruct((S, D), bf16),
        in_specs=[any_spec] * 8,
        out_specs=any_spec,
        scratch_shapes=scratch,
        compiler_params=pltpu.CompilerParams(vmem_limit_bytes=110 * 1024 * 1024),
    )(A_q.reshape(S, D), A_k.reshape(S, D), A_v.reshape(S, D), A_shift_k.T, A_ssm_k,
      A_ssm_D, B_wqkv, B_wo)
    return out.reshape(1, S, D)
```
